```python
import jax
import jax.numpy as jnp

def _softmax(x, axis=-1):
    return jax.nn.softmax(x, axis=axis)
def _gelu(x):
    return jax.nn.gelu(x, approximate=True)
def _silu(x):
    return jax.nn.silu(x)
def _sigmoid(x):
    return jax.nn.sigmoid(x)
def _layernorm(x, axis=-1, eps=1e-5):
    m = jnp.mean(x, axis=axis, keepdims=True)
    v = jnp.var(x, axis=axis, keepdims=True)
    return (x - m) / jnp.sqrt(v + eps)
def _scatter_add(tgt, idx, src, axis=0):
    return tgt.at[idx].add(src)
def _segment_sum(src, seg, n):
    return jax.ops.segment_sum(src, seg, n)
class _Rng:
    def __init__(self, key):
        self._k = key
    def _next(self):
        self._k, sub = jax.random.split(self._k)
        return sub
    def normal(self, shape):
        return jax.random.normal(self._next(), shape, dtype=jnp.bfloat16)
    def randint(self, lo, hi, shape):
        return jax.random.randint(self._next(), shape, lo, hi, dtype=jnp.int32)
    def uniform(self, shape, lo=0.0, hi=1.0):
        return jax.random.uniform(self._next(), shape, jnp.bfloat16, lo, hi)
    def permutation(self, n):
        return jax.random.permutation(self._next(), n)


kernel_name = 'recurrent_scan__sliding_local_dilated__moe_arch_mod__prompt'

def setup_inputs():
    _rng = _Rng(jax.random.key(int.from_bytes(__import__("os").urandom(4), "little")))
    _w = (lambda a: (lambda t: t.astype(jnp.bfloat16) if jnp.issubdtype(t.dtype, jnp.floating) else t)(jnp.asarray(a)))
    def _A_setup():
        B, S, D = 1, 2048, 640
        return {
            "x": _w((lambda *s: _rng.normal(s) * 0.05)(B, S, D)),
            "wqkv": _w((lambda *s: _rng.normal(s) * 0.05)(D, 3 * D)),
            "wo": _w((lambda *s: _rng.normal(s) * 0.05)(D, D)),
        }
    _A_in = _A_setup()

    def _B_setup():
        B, S, D, F, C = 1, 2048, 640, 1728, 2
        return {
            "x": _w((lambda *s: _rng.normal(s) * 0.05)(B, S, D)),
            "w_r": _w((lambda *s: _rng.normal(s) * 0.05)(D)),
            "w_gate": _w((lambda *s: _rng.normal(s) * 0.05)(D, F)),
            "w_up": _w((lambda *s: _rng.normal(s) * 0.05)(D, F)),
            "w_down": _w((lambda *s: _rng.normal(s) * 0.05)(F, D)),
        }
    _B_in = _B_setup()

    return {
        "A_x": _A_in["x"],
        "A_wqkv": _A_in["wqkv"],
        "A_wo": _A_in["wo"],
        "B_x": _B_in["x"],
        "B_w_r": _B_in["w_r"],
        "B_w_gate": _B_in["w_gate"],
        "B_w_up": _B_in["w_up"],
        "B_w_down": _B_in["w_down"],
    }

def reference(A_x, A_wqkv, A_wo, B_x, B_w_r, B_w_gate, B_w_up, B_w_down):
    def _A_ref(x, wqkv, wo):
        B, S, D = x.shape
        H = 32; Dh = D // H
        W, dil = 8, 2
        qkv = (lambda x, *d: x.transpose(*d))((x @ wqkv).reshape(B, S, 3, H, Dh), 2, 0, 3, 1, 4)
        q, k, v = qkv[0], qkv[1], qkv[2]
        scale = Dh ** -0.5
        pos = jnp.arange(S)
        off = jnp.arange(W) * dil
        idx = pos[:, None] - off[None, :]
        mask = idx >= 0
        idx_c = jnp.where(mask, idx, 0).reshape(-1)
        kg = k[:, :, idx_c, :].reshape(B, H, S, W, Dh)
        vg = v[:, :, idx_c, :].reshape(B, H, S, W, Dh)
        logits = jnp.einsum("bhsd,bhswd->bhsw", q, kg) * scale
        logits = jnp.where(mask[None, None, :, :], logits, -1e9)
        attn = _softmax(logits, axis=-1)
        o = jnp.einsum("bhsw,bhswd->bhsd", attn, vg)
        return (lambda x, *d: x.transpose(*d))(o, 0, 2, 1, 3).reshape(B, S, D) @ wo

    def _B_ref(x, w_r, w_gate, w_up, w_down):
        B, S, D = x.shape
        C = 2
        r = x @ w_r
        idx = jnp.argsort(-r, axis=-1)[:, :C]
        idx_e = jnp.repeat(idx.reshape(B, C, 1), D, axis=2)
        x_sel = jnp.take_along_axis(x, idx_e, axis=1)
        g = _silu(x_sel @ w_gate)
        u = x_sel @ w_up
        y = (g * u) @ w_down
        r_sel = _sigmoid(jnp.take_along_axis(r, idx, axis=1))
        y = y * r_sel.reshape(B, C, 1)
        b_off = (jnp.arange(B) * S).reshape(B, 1)
        flat_idx = (idx + b_off).reshape(B * C)
        zero = (x * 0.0).reshape(B * S, D)
        upd = _scatter_add(zero, flat_idx, y.reshape(B * C, D), axis=0)
        return x + upd.reshape(B, S, D)

    x = A_x
    xn = _layernorm(x, axis=-1)
    s = _A_ref(xn, A_wqkv, A_wo)
    g = _silu(_B_ref(xn, B_w_r, B_w_gate, B_w_up, B_w_down))
    return x + s * g
```

```python
import functools

import jax
import jax.numpy as jnp
import numpy as np
from jax import lax
from jax.experimental import pallas as pl
from jax.experimental.pallas import tpu as pltpu

S, D, F = 2048, 640, 1728
H, DH, W, DIL = 32, 20, 8, 2
NT = D // 128
HALO = 16
BF = jnp.bfloat16
F32 = jnp.float32
U32 = jnp.uint32
LOG2E = 1.4426950408889634
NEG = -998244352.0
EPS = 1.0013580322265625e-05


M = 128
NC = S // M
XC = 256
FFN_AT = 9
A1 = 0.55
MODE = 0


def _rb(x):
    return x.astype(BF).astype(F32)


def _lo(u):
    return lax.bitcast_convert_type(u << 16, F32)


def _hi(u):
    return lax.bitcast_convert_type(u & np.uint32(0xFFFF0000), F32)


def _nt(a, b):
    return lax.dot_general(a, b, (((1,), (1,)), ((), ())), preferred_element_type=F32)


def _pk(x):
    return pltpu.bitcast(x.astype(BF), U32)


def _up(u):
    return pltpu.bitcast(u, BF)


def _silu(x):
    h = x * 0.5
    return h * jnp.tanh(h) + h


def _sum(xs):
    return functools.reduce(jnp.add, xs)


def _tiles(x):
    return [x[:, t * 128:(t + 1) * 128] for t in range(x.shape[1] // 128)]


class _Pipe:
    def __init__(self, make, n):
        self.make, self.n, self.started, self.done, self.live = make, n, 0, 0, []

    def step(self, start):
        for g in list(self.live):
            if next(g, "end") == "end":
                self.live.remove(g)
                self.done += 1
        if start and self.started < self.n:
            g = self.make(self.started)
            self.started += 1
            next(g)
            self.live.append(g)


def _kernel(x_hbm, wqkv_hbm, wo_hbm, wr_hbm, wg_hbm, wu_hbm, wd_hbm, out_hbm,
            xb, wraw, woraw, wrb, wg, wu, wd, stage, wt, wop, xn, gin, qs, ks, vs,
            ob, outb, xsem, wsem, osem):
    def xcopy(c):
        return pltpu.make_async_copy(x_hbm.at[pl.ds(c * XC, XC)], xb.at[pl.ds(c * XC, XC)], xsem.at[c])

    def wcopy(m):
        return pltpu.make_async_copy(wqkv_hbm.at[:, pl.ds(m * D, D)], wraw.at[m], wsem.at[m])

    def ocopy(c):
        return pltpu.make_async_copy(outb.at[pl.ds(c * M, M)], out_hbm.at[pl.ds(c * M, M)], osem.at[c])

    wocopy = pltpu.make_async_copy(wo_hbm, woraw, wsem.at[3])
    wrcopy = pltpu.make_async_copy(wr_hbm, wrb, wsem.at[4])
    wgcopy = pltpu.make_async_copy(wg_hbm, wg, wsem.at[5])
    wucopy = pltpu.make_async_copy(wu_hbm, wu, wsem.at[6])
    wdcopy = pltpu.make_async_copy(wd_hbm, wd, wsem.at[7])

    wcopy(1).start()
    wrcopy.start()
    xcopy(0).start()
    wcopy(2).start()
    wcopy(0).start()
    for c in range(1, S // XC):
        xcopy(c).start()
    wocopy.start()
    wgcopy.start()
    wucopy.start()
    wdcopy.start()

    def permute_rows(t, dst, col):
        for d2 in range(DH // 2):
            u = stage[t, pl.ds(d2, H, stride=DH // 2), :]
            dst[pl.ds(H * d2, H // 2), pl.ds(col, 128)] = _pk(_lo(u))
            dst[pl.ds(H * d2 + H // 2, H // 2), pl.ds(col, 128)] = _pk(_hi(u))

    def prep_w(m, kt):
        blk = wraw[m, pl.ds(kt * 128, 128), :]
        stage[m * NT + kt] = pltpu.bitcast(blk.T, U32)
        permute_rows(m * NT + kt, wt.at[m], kt * 128)

    def prep_wo(t):
        stage[3 * NT + t] = pltpu.bitcast(woraw[:, pl.ds(t * 128, 128)], U32)
        permute_rows(3 * NT + t, wop, t * 128)

    lane = lax.broadcasted_iota(jnp.int32, (16, 128), 1)
    st = {"r": jnp.zeros((16, 128), F32), "x": 0}

    def ln(i):
        r0 = 16 * i
        if r0 // XC >= st["x"]:
            xcopy(st["x"]).wait()
            st["x"] += 1
        x = _tiles(xb[pl.ds(r0, 16), :].astype(F32))
        s = _sum(x)
        tot = jnp.sum(s, axis=1, keepdims=True)
        ml = s * (1.0 / NT)
        m2 = _sum([(a - ml) * (a - ml) for a in x])
        yield
        mean = tot * (1.0 / D)
        dm = ml - mean
        tot = jnp.sum(m2 + (dm * dm) * float(NT), axis=1, keepdims=True)
        yield
        sd = _rb(jnp.sqrt(_rb(_rb(tot * (1.0 / D)) + EPS)))
        x = xb[pl.ds(r0, 16), :].astype(F32)
        y = (_rb(x - _rb(mean)) * (1.0 / sd)).astype(BF)
        xn[pl.ds(r0 // 2, 8), :] = pltpu.bitcast(y, U32)
        gin[pl.ds(r0 // 2, 8), :] = pltpu.bitcast(y, U32)
        r = jnp.sum(_sum(_tiles(y.astype(F32) * st["wr"])), axis=1, keepdims=True)
        yield
        st["r"] = jnp.where(lane == i, r, st["r"])

    def qkv(c, m, t):
        y = _nt(_up(xn[pl.ds(c * M // 2, M // 2), :]), _up(wt[m, pl.ds(t * 64, 64), :]))
        if m == 0:
            qs[t, pl.ds(c * M, M), :] = y * (DH ** -0.5 * LOG2E)
        else:
            dst = ks if m == 1 else vs
            dst[t, pl.ds(HALO + c * M, M), :] = y
            if c == 0:
                dst[t, pl.ds(0, HALO), :] = jnp.broadcast_to(y[0:1, :], (HALO, 128))

    def attn(g):
        r0 = 8 * g
        q = [qs[t, pl.ds(r0, 8), :] for t in range(NT)]
        p = []
        for w in range(W):
            rows = pl.ds(HALO + r0 - DIL * w, 8)
            p.append(_sum([q[t] * ks[t, rows, :] for t in range(NT)]))
        rl = [pltpu.roll(a, 64, 1) for a in p]
        yield
        p = [a + b for a, b in zip(p, rl)]
        rl = [pltpu.roll(a, 32, 1) for a in p]
        yield
        p = [a + b for a, b in zip(p, rl)]
        for w in range(W):
            if r0 < DIL * w:
                row = lax.broadcasted_iota(jnp.int32, (8, 128), 0) + r0
                p[w] = jnp.where(row >= DIL * w, p[w], NEG * LOG2E)
        mx = functools.reduce(jnp.maximum, p)
        e = [jnp.exp2(a - mx) for a in p]
        inv = pltpu.reciprocal(_sum(e), full_range=False)
        o = [_sum([e[w] * vs[t, pl.ds(HALO + r0 - DIL * w, 8), :] for w in range(W)]) * inv
             for t in range(NT)]
        if g % 2 == 0:
            st["o"] = o
        else:
            for t in range(NT):
                ob[pl.ds(r0 // 2 - 4, 8), pl.ds(t * 128, 128)] = _pk(
                    jnp.concatenate([st["o"][t], o[t]], axis=0))

    def proj(c, t):
        rows, half, cols = pl.ds(c * M, M), pl.ds(c * M // 2, M // 2), pl.ds(t * 128, 128)
        s = jnp.dot(_up(ob[half, :]), _up(wop[:, cols]), preferred_element_type=F32)
        g = _silu(_up(gin[half, cols]).astype(F32))
        outb[rows, cols] = (xb[rows, cols].astype(F32) + s * g).astype(BF)
        if t == NT - 1:
            ocopy(c).start()

    def ffn():
        r = _rb(st["r"])
        key = jnp.where(r != r, -jnp.inf, r)
        tok = lane * 16 + lax.broadcasted_iota(jnp.int32, (16, 128), 0)
        picks = []
        for _ in range(2):
            top = jnp.max(key, keepdims=True)
            cand = key == top
            if picks:
                cand = cand & (tok != picks[0][0])
            idx = jnp.min(jnp.where(cand, tok, S), keepdims=True)
            val = jnp.sum(jnp.where(tok == idx, r, 0.0), keepdims=True)
            picks.append((idx, val))
            key = jnp.where(tok == idx, -jnp.inf, key)
        base = [pl.multiple_of((jnp.squeeze(i) // 16) * 8, 8) for i, _ in picks]
        yield
        wgcopy.wait()
        wucopy.wait()
        row = lax.broadcasted_iota(jnp.int32, (16, D), 0)
        sel = [jnp.sum(jnp.where(row == i % 16, _up(xn[pl.ds(b, 8), :]).astype(F32), 0.0),
                       axis=0, keepdims=True) for (i, _), b in zip(picks, base)]
        xs = jnp.where(row == 0, sel[0], sel[1]).astype(BF)
        yield
        hid = []
        NF = -(-F // 128)
        for n0 in range(0, NF, 4):
            ns = range(n0, min(n0 + 4, NF))
            gu = []
            for wref in (wg, wu):
                lo, hi = n0 * 128, min((n0 + 4) * 128, F)
                rem = _nt(xs[:, 512:], wref[pl.ds(lo, hi - lo), pl.ds(512, 128)])
                yield
                part = []
                for n in ns:
                    lo1, hi1 = n * 128, min((n + 1) * 128, F)
                    part.append(_nt(xs[:, :512], wref[pl.ds(lo1, hi1 - lo1), pl.ds(0, 512)])
                                + rem[:, lo1 - lo:hi1 - lo])
                    yield
                gu.append(part)
            for g, u in zip(*gu):
                hid.append((_rb(_silu(_rb(g))) * _rb(u)).astype(BF))
        wdcopy.wait()
        y = None
        for n in range(NF):
            lo1, hi1 = n * 128, min((n + 1) * 128, F)
            a = jnp.dot(hid[n], wd[pl.ds(lo1, hi1 - lo1), pl.ds(0, 512)], preferred_element_type=F32)
            y = a if y is None else y + a
            yield
        y4 = None
        for n0 in range(0, NF, 4):
            lo, hi = n0 * 128, min((n0 + 4) * 128, F)
            a = jnp.dot(jnp.concatenate(hid[n0:n0 + 4], axis=1), wd[pl.ds(lo, hi - lo), pl.ds(512, 128)],
                        preferred_element_type=F32)
            y4 = a if y4 is None else y4 + a
            yield
        y = _rb(jnp.concatenate([y, y4], axis=1))
        for j, (idx, val) in enumerate(picks):
            upd = _rb(y[j:j + 1] * _rb(jax.nn.sigmoid(val)))
            cur = _up(gin[pl.ds(base[j], 8), :]).astype(F32)
            gin[pl.ds(base[j], 8), :] = _pk(jnp.where(row == idx % 16, cur + upd, cur))

    lnp = _Pipe(ln, S // 16)
    atp = _Pipe(attn, S // 8)
    GPC = M // 8

    wcopy(1).wait()
    for kt in range(NT):
        prep_w(1, kt)
    wrcopy.wait()
    st["wr"] = wrb[...].astype(F32).reshape(1, D)
    gens = [ln(i) for i in range(M // 16)]
    for _ in range(4):
        for g in gens:
            next(g, None)
    lnp.started = lnp.done = M // 16

    order = []
    for c in range(NC):
        order += [("qkv", c, m, t) for m in (1, 2, 0) for t in range(NT)]
    nffn = 60
    first = order[:FFN_AT * 15 + nffn]
    rest = order[FFN_AT * 15 + nffn:]
    projs = [("proj", c, t) for c in range(NC) for t in range(NT)]
    tail = 3 * NT
    merged = []
    a, b = rest, projs[:-tail]
    i = j = 0
    while i < len(a) or j < len(b):
        if j >= len(b) or (i < len(a) and i * len(b) < j * len(a)):
            merged += a[i:i + NT]; i += NT
        else:
            merged += b[j:j + NT]; j += NT
    order = first + merged + projs[-tail:]

    extra = {}
    extra[0] = [wcopy(2).wait]
    for kt in range(NT):
        extra.setdefault(kt, []).append(functools.partial(prep_w, 2, kt))
    extra[NT] = [wcopy(0).wait]
    for kt in range(NT):
        extra.setdefault(NT + kt, []).append(functools.partial(prep_w, 0, kt))
    extra[100] = [wocopy.wait]
    for t in range(NT):
        extra.setdefault(100 + t, []).append(functools.partial(prep_wo, t))

    ffng = ffn()
    ffn_done = False
    ready = 0
    credit = 0.0
    for slot, task in enumerate(order):
        if task[0] == "qkv":
            _, c, m, t = task
            while lnp.done < (c + 1) * M // 16:
                lnp.step(True)
            qkv(c, m, t)
        else:
            _, c, t = task
            while not ffn_done:
                ffn_done = next(ffng, "end") == "end"
            while atp.done < (c + 1) * GPC:
                atp.step(atp.started < ready)
            proj(c, t)
        if slot >= FFN_AT * 15 and not ffn_done:
            while lnp.done < lnp.n:
                lnp.step(True)
            ffn_done = next(ffng, "end") == "end"
        lnp.step(True)
        if lnp.done < lnp.n:
            credit += A1
        else:
            left = len(order) - NT - 3 - slot
            credit += (atp.n - atp.started) / max(left, 1)
        k = 0
        while credit >= 1 and atp.started < ready:
            credit -= 1
            atp.step(True)
            k += 1
        if k == 0:
            atp.step(False)
        credit = min(credit, 1.0)
        for f in extra.get(slot, []):
            f()
        if task[0] == "qkv" and task[2:] == (0, NT - 1):
            ready = (task[1] + 1) * GPC
    for c in range(NC):
        ocopy(c).wait()


@jax.jit
def pallas_recurrent_scan__sliding_local_dilated__moe_arch_mod__prompt_kernel(
    A_x, A_wqkv, A_wo, B_x, B_w_r, B_w_gate, B_w_up, B_w_down,
):
    del B_x
    hbm = pl.BlockSpec(memory_space=pltpu.HBM)
    V = pltpu.VMEM
    out = pl.pallas_call(
        _kernel,
        in_specs=[hbm] * 7,
        out_specs=hbm,
        out_shape=jax.ShapeDtypeStruct((S, D), BF),
        scratch_shapes=[
            V((S, D), BF),
            V((3, D, D), BF),
            V((D, D), BF),
            V((D,), BF),
            V((F, D), BF), V((F, D), BF), V((F, D), BF),
            V((4 * NT, D // 2, 128), U32),
            V((3, D // 2, D), U32),
            V((D // 2, D), U32),
            V((S // 2, D), U32),
            V((S // 2, D), U32),
            V((NT, S, 128), F32),
            V((NT, HALO + S, 128), F32),
            V((NT, HALO + S, 128), F32),
            V((S // 2, D), U32),
            V((S, D), BF),
            pltpu.SemaphoreType.DMA((S // XC,)),
            pltpu.SemaphoreType.DMA((8,)),
            pltpu.SemaphoreType.DMA((NC,)),
        ],
        compiler_params=pltpu.CompilerParams(vmem_limit_bytes=100 << 20),
        name="fused",
    )(A_x.reshape(S, D), A_wqkv, A_wo, B_w_r, B_w_gate.T, B_w_up.T, B_w_down)
    return out.reshape(1, S, D)
```

```python
import functools

import jax
import jax.numpy as jnp
import numpy as np
from jax import lax
from jax.experimental import pallas as pl
from jax.experimental.pallas import tpu as pltpu

S, D, F = 2048, 640, 1728
H, DH, W, DIL = 32, 20, 8, 2
NT = D // 128
NF = -(-F // 128)
HALO = 8
BF = jnp.bfloat16
F32 = jnp.float32
U32 = jnp.uint32
LOG2E = 1.4426950408889634
NEG = -998244352.0
EPS = 1.0013580322265625e-05


M = 128
NC = S // M
XCUT = (0, 256, 512, 1024, 2048)
FP = 1
PAIR = 2
F0 = 50
FFN_AT = 165
LN_DUE = 140
P0 = 1
PO = 1
TAIL = 3
LAG = 2
TIE = 1
SCOPE = 0


def _pack(a, b):
    return pltpu.pack_elementwise([a, b], packed_dtype=BF)


def _unpack(u):
    return [pltpu.unpack_elementwise(u, index=i, packed_dtype=BF, unpacked_dtype=F32)
            for i in range(2)]


def _rb2(a, b):
    return _unpack(_pack(a, b))


def _rb4(v):
    return _rb2(v[0], v[1]) + _rb2(v[2], v[3])


def _rb(x):
    return x.astype(BF).astype(F32)


def _nt(a, b):
    return lax.dot_general(a, b, (((1,), (1,)), ((), ())), preferred_element_type=F32)


def _nn(a, b):
    return jnp.dot(a, b, preferred_element_type=F32)


def _bf(u):
    return pltpu.bitcast(u, BF)


def _silu(x):
    h = x * 0.5
    return h * jnp.tanh(h) + h


def _sum(xs):
    return functools.reduce(jnp.add, xs)


def _advance(g):
    return next(g, "end") == "end"


class _Pipe:
    def __init__(self, make, n, last):
        self.last = last
        self.make, self.n, self.started, self.done, self.live = make, n, 0, 0, []

    def step(self, start):
        live = self.live
        self.live = []
        rest = [e for e in live if e[0] < self.last]
        for e in live:
            if e[0] == self.last:
                _advance(e[1])
                self.done += 1
        if start and self.started < self.n:
            rest.append([0, self.make(self.started)])
            self.started += 1
        for e in reversed(rest):
            next(e[1])
            e[0] += 1
        self.live = rest


class _Copies:
    def __init__(self, pairs, sem):
        self.cs = [pltpu.make_async_copy(a, b, sem) for a, b in pairs]

    def start(self, pri):
        for c in self.cs:
            c.start(priority=pri)

    def wait(self):
        for c in self.cs:
            c.wait()


def _kernel(x_hbm, wqkv_hbm, wo_hbm, wr_hbm, wg_hbm, wu_hbm, wd_hbm, out_hbm,
            xb, wraw, wrb, wf, stage, wt, wop, xn, gate, qs, ks, vs, ob, outb, wrf,
            xsem, wsem, osem):
    col = lambda t: pl.ds(t * 128, 128)
    xu = xb.bitcast(U32)

    xcopy = [_Copies([(x_hbm.at[pl.ds(a, b - a), col(t)], xb.at[t, pl.ds(a, b - a)])
                      for t in range(NT)], xsem.at[i])
             for i, (a, b) in enumerate(zip(XCUT[:-1], XCUT[1:]))]

    def wcopy(m, a, b, sem):
        return _Copies([(wqkv_hbm.at[pl.ds(a, b - a), pl.ds(m * D, D)],
                         wraw.at[m, pl.ds(a, b - a)])], wsem.at[sem])

    kcopy = [wcopy(1, 0, 384, 0), wcopy(1, 384, D, 1)]
    vcopy = wcopy(2, 0, D, 2)
    qcopy = wcopy(0, 0, D, 3)
    wocopy = _Copies([(wo_hbm, wraw.at[3])], wsem.at[4])
    wrcopy = _Copies([(wr_hbm, wrb)], wsem.at[5])
    fcopy = _Copies([(w.at[pl.ds(j * F // FP, F // FP)], wf.at[i, pl.ds(j * F // FP, F // FP)])
                     for i, w in enumerate((wg_hbm, wu_hbm, wd_hbm)) for j in range(FP)], wsem.at[6])
    ocopy = _Copies([(outb.at[pl.ds(c * M, M), col(t)], out_hbm.at[pl.ds(c * M, M), col(t)])
                     for c in range(NC) for t in range(NT)], osem)

    for c in (wrcopy, xcopy[0], kcopy[0], kcopy[1]):
        c.start(P0)

    def permute_rows(src, dst, t):
        for d2 in range(DH // 2):
            u = src[pl.ds(d2, H // 2, stride=DH), :]
            v = src[pl.ds(d2 + DH // 2, H // 2, stride=DH), :]
            dst[pl.ds(H * d2, H // 2), col(t)] = (u & np.uint32(0xFFFF)) | (v << 16)
            dst[pl.ds(H * d2 + H // 2, H // 2), col(t)] = (u >> 16) | (v & np.uint32(0xFFFF0000))

    def prep_a(m, kt):
        stage[m * NT + kt] = pltpu.bitcast(wraw[m, pl.ds(kt * 128, 128), :].T, U32)

    def prep_b(m, kt):
        permute_rows(stage.at[m * NT + kt], wt.at[m], kt)

    def prep_wo(t):
        stage[3 * NT + t] = pltpu.bitcast(wraw[3, :, col(t)], U32)
        permute_rows(stage.at[3 * NT + t], wop, t)

    lane = lax.broadcasted_iota(jnp.int32, (8, 128), 1)
    st = {"r": [jnp.zeros((8, 128), F32)] * 2}

    def tie(v, age=-1):
        if not TIE or "tok" not in st:
            return v
        n = v.shape[1]
        return jnp.where(st["never"][:, :n], lax.bitcast_convert_type(st["tok"][age], v.dtype)[:, :n], v)

    def ln(i):
        def load(t):
            return (_unpack(xu[t, pl.ds(16 * i, 8, stride=2), :])
                    + _unpack(xu[t, pl.ds(16 * i + 1, 8, stride=2), :]))

        x = [load(t) for t in range(NT)]
        x[0] = [tie(a) for a in x[0]]
        x = list(zip(*x))
        tot, ml, m2 = [], [], []
        for xs in x:
            s = _sum(xs)
            tot.append(jnp.sum(s, axis=1, keepdims=True))
            ml.append(s * (1.0 / NT))
            m2.append(_sum([(a - ml[-1]) * (a - ml[-1]) for a in xs]))
        yield
        mean = [jnp.broadcast_to(a, (8, 128)) * (1.0 / D) for a in tot]
        tot = [jnp.sum(b + ((a - m) * (a - m)) * float(NT), axis=1, keepdims=True)
               for a, b, m in zip(ml, m2, mean)]
        mean = [_pack(mean[0], mean[1]), _pack(mean[2], mean[3])]
        yield
        var = _rb4([jnp.broadcast_to(a, (8, 128)) * (1.0 / D) for a in tot])
        sd = _rb4([jnp.sqrt(a) for a in _rb4([a + EPS for a in var])])
        inv = [1.0 / a for a in sd]
        mean = _unpack(mean[0]) + _unpack(mean[1])
        r = None
        c, j = divmod(i, M // 32)
        for t in range(NT):
            y = [a * b for a, b in zip(_rb4([a - m for a, m in zip(load(t), mean)]), inv)]
            ye, yo = _pack(y[0], y[2]), _pack(y[1], y[3])
            xn[pl.ds(c * M // 2 + 8 * j, 8), col(t)] = ye
            xn[pl.ds(c * M // 2 + M // 4 + 8 * j, 8), col(t)] = yo
            y = [b for a in zip(_unpack(ye), _unpack(yo)) for b in a]
            gate[t, pl.ds(16 * i, 8, stride=2), :] = _pack(_silu(y[0]), _silu(y[1]))
            gate[t, pl.ds(16 * i + 1, 8, stride=2), :] = _pack(_silu(y[2]), _silu(y[3]))
            w = wrf[:, col(t)]
            a = [a * w for a in y]
            r = a if r is None else [b + e for b, e in zip(r, a)]
        r = [jnp.sum(a, axis=1, keepdims=True) for a in r]
        st["xn"] = 32 * (i + 1)
        yield
        k = i // 32
        for s in range(4):
            st["r"][k] = jnp.where(lane == (4 * i + s) % 128, r[s], st["r"][k])

    def qkv(c, m, t):
        y = _nt(_bf(xn[pl.ds(c * M // 2, M // 2), :]), _bf(wt[m, pl.ds(t * 64, 64), :]))
        st.setdefault("tok", []).append(y[-8:])
        yield
        for p in range(2):
            yp = y[p * M // 2:(p + 1) * M // 2]
            if m == 0:
                qs[t, p, pl.ds(c * M // 2, M // 2), :] = yp * (DH ** -0.5 * LOG2E)
            else:
                dst = ks if m == 1 else vs
                dst[t, p, pl.ds(HALO + c * M // 2, M // 2), :] = yp
                if c == 0:
                    dst[t, p, pl.ds(0, HALO), :] = jnp.broadcast_to(y[0:1, :], (HALO, 128))

    def attn(g):
        jb, par = divmod(g, 2)
        r0 = 8 * jb
        q = [tie(qs[t, par, pl.ds(r0, 8), :]) for t in range(NT)]
        p = []
        for w in range(W):
            rows = pl.ds(HALO + r0 - w, 8)
            p.append(_sum([q[t] * ks[t, par, rows, :] for t in range(NT)]))
        rl = [pltpu.roll(a, 64, 1) for a in p]
        yield
        p = [a + b for a, b in zip(p, rl)]
        rl = [pltpu.roll(a, 32, 1) for a in p]
        yield
        p = [a + b for a, b in zip(p, rl)]
        if jb == 0:
            row = lax.broadcasted_iota(jnp.int32, (8, 128), 0)
            p = [jnp.where(row >= w, a, NEG * LOG2E) for w, a in enumerate(p)]
        mx = functools.reduce(jnp.maximum, p)
        e = [jnp.exp2(a - mx) for a in p]
        inv = pltpu.reciprocal(_sum(e), full_range=False)
        o = [_sum([e[w] * vs[t, par, pl.ds(HALO + r0 - w, 8), :] for w in range(W)]) * inv
             for t in range(NT)]
        if par == 0:
            st["o"] = o
        else:
            for t in range(NT):
                ob[pl.ds(r0, 8), col(t)] = _pack(st["o"][t], o[t])

    def proj(c, t):
        half = pl.ds(c * M // 2, M // 2)
        s = _nn(_bf(ob[half, :]), _bf(wop[:, col(t)]))
        st["tok"].append(s[-8:])
        yield
        g = _bf(gate[t, half, :]).astype(F32)
        outb[pl.ds(c * M, M), col(t)] = (_bf(xu[t, half, :]).astype(F32) + s * g).astype(BF)
        ocopy.cs[c * NT + t].start(priority=PO)

    def route():
        r = jnp.concatenate(_rb2(*st["r"]), axis=1)
        key = jnp.where(r != r, -jnp.inf, r)
        slot = lax.broadcasted_iota(jnp.int32, (8, 256), 1)
        tok = (slot >> 2) * 32 + (slot & 3) + 4 * lax.broadcasted_iota(jnp.int32, (8, 256), 0)
        picks = []
        for _ in range(2):
            top = jnp.max(key, keepdims=True)
            yield
            cand = key == top
            if picks:
                cand = cand & (tok != picks[0][0])
            idx = jnp.min(jnp.where(cand, tok, S), keepdims=True)
            yield
            val = jnp.sum(jnp.where(tok == idx, r, 0.0), keepdims=True)
            picks.append((idx, val))
            key = jnp.where(tok == idx, -jnp.inf, key)
        sidx = [jnp.squeeze(i) for i, _ in picks]
        base = [pl.multiple_of((i >> 4) * 8, 8) for i in sidx]
        src = [pl.multiple_of((i >> 7) * 64 + (i & 1) * 32 + ((i >> 5) & 3) * 8, 8) for i in sidx]
        yield
        row = lax.broadcasted_iota(jnp.int32, (16, 128), 0)
        xs = []
        for t in range(NT):
            sel = [jnp.sum(jnp.where(row == ((i >> 1) & 15),
                                     _bf(xn[pl.ds(b, 8), col(t)]).astype(F32), 0.0),
                           axis=0, keepdims=True) for (i, _), b in zip(picks, src)]
            sel = [jnp.broadcast_to(a, (8, 128)) for a in sel]
            xs.append(_pack(sel[0], sel[1]))
        st["route"] = (picks, base, xs)

    def ffn():
        picks, base, xs = st["route"]
        span = lambda a, b: pl.ds(a * 128, min(b * 128, F) - a * 128)
        lhs = lambda us: jnp.concatenate([_bf(tie(u, -3)) for u in us], axis=1)
        hid = []
        for n0 in range(0, NF, 4):
            n1 = min(n0 + 4, NF)
            gu = []
            for i in range(2):
                rem = _nt(lhs(xs[4:]), wf[i, span(n0, n1), col(4)])[:8]
                yield
                part = []
                for n in range(n0, n1):
                    a = _nt(lhs(xs[:4]), wf[i, span(n, n + 1), pl.ds(0, 512)])[:8]
                    part.append(a + rem[:, (n - n0) * 128:(n - n0) * 128 + a.shape[1]])
                    yield
                gu.append(part)
            for g, u in zip(*gu):
                g, u = _rb2(g, u)
                a = _rb2(_silu(g), u)[0] * u
                hid.append(_pack(a, a))
        y = None
        for n in range(NF):
            a = _nn(lhs(hid[n:n + 1]), wf[2, span(n, n + 1), pl.ds(0, 512)])[:8]
            y = a if y is None else y + a
            yield
        y4 = None
        for n0 in range(0, NF, 4):
            a = _nn(lhs(hid[n0:n0 + 4]),
                    wf[2, span(n0, min(n0 + 4, NF)), col(4)])[:8]
            y4 = a if y4 is None else y4 + a
            yield
        y = _rb(jnp.concatenate([y, y4], axis=1))
        row = lax.broadcasted_iota(jnp.int32, (8, 128), 0)
        for j, (idx, val) in enumerate(picks):
            upd = _rb(y[2 * j:2 * j + 1] * _rb(jax.nn.sigmoid(val)))
            for t in range(NT):
                xsel = _unpack(xs[t])[j]
                g = _silu(_rb(xsel + upd[:, t * 128:(t + 1) * 128]))
                cur = _unpack(gate[t, pl.ds(base[j], 8), :])
                gate[t, pl.ds(base[j], 8), :] = _pack(
                    *[jnp.where(2 * row + p == (idx & 15), g, a) for p, a in enumerate(cur)])

    lnp = _Pipe(ln, S // 32, 3)
    atp = _Pipe(attn, S // 8, 2)
    GPC = M // 8

    import contextlib
    scope = contextlib.ExitStack()
    if SCOPE:
        scope.enter_context(jax.named_scope('pro'))
    wrcopy.wait()
    xcopy[0].wait()
    wrf[...] = jnp.broadcast_to(wrb[...].astype(F32).reshape(1, D), (8, D))
    st["never"] = (lax.bitcast_convert_type(wrf[:, col(0)], U32) & np.uint32(0xFFFF)) != 0
    while lnp.done < XCUT[1] // 32:
        lnp.step(lnp.started < XCUT[1] // 32)
    for cp, kts in zip(kcopy, ((0, 1, 2), (3, 4))):
        cp.wait()
        if kts[0] == 0:
            xcopy[1].start(P0)
            vcopy.start(P0)
        for kt in kts:
            prep_a(1, kt)
        for kt in kts:
            prep_b(1, kt)

    if SCOPE:
        scope.close()
        scope.enter_context(jax.named_scope('s000'))
    tiles = lambda c, m: [("qkv", c, m, t) for t in range(NT)]
    order = [a for m in (1, 2, 0) for c in range(4) for a in tiles(c, m)]
    order += [a for c in range(4, NC) for m in (1, 2, 0) for a in tiles(c, m)]
    nffn = 60
    a = order[FFN_AT + nffn:]
    order = order[:FFN_AT + nffn]
    projs = [("proj", c, t) for c in range(NC) for t in range(NT)]
    b = projs[:-TAIL * NT]
    i = j = 0
    while i < len(a) or j < len(b):
        if j >= len(b) or (i < len(a) and i * len(b) < j * len(a)):
            order += a[i:i + NT]
            i += NT
        else:
            order += b[j:j + NT]
            j += NT
    order += projs[-TAIL * NT:]

    need = {t[1]: s for s, t in enumerate(order) if t[0] == "proj" and t[2] == 0}
    avail = {t[1]: s for s, t in enumerate(order) if t[0] == "qkv" and t[2:] == (0, NT - 1)}

    P = functools.partial
    waits = {1: [xcopy[1]], 13: [vcopy], 30: [qcopy, xcopy[2]], 58: [xcopy[3], wocopy],
             FFN_AT: [fcopy]}
    starts = {1: [qcopy, xcopy[2]], 13: [xcopy[3], wocopy], F0: [fcopy]}
    xready = {1: (XCUT[2], 12), 30: (XCUT[3], 58), 58: (XCUT[4], LN_DUE)}
    extra = {}
    for kt in range(NT):
        extra.setdefault(13 + kt, []).append(P(prep_a, 2, kt))
        extra.setdefault(14 + kt, []).append(P(prep_b, 2, kt))
        extra.setdefault(30 + kt, []).append(P(prep_a, 0, kt))
        extra.setdefault(32 + kt, []).append(P(prep_b, 0, kt))
        extra.setdefault(FFN_AT + 10 * kt, []).append(P(prep_wo, kt))

    routeg, ffng = route(), ffn()
    route_done = ffn_done = False
    xrows, xdue, lcredit = XCUT[1], 0, 0.0
    credit = 0.0
    for slot, task in enumerate(order):
        if task[0] == "qkv":
            while st["xn"] < (task[1] + 1) * M:
                lnp.step(lnp.started < xrows // 32)
            g = qkv(*task[1:])
        else:
            while not ffn_done:
                ffn_done = _advance(ffng)
            while atp.done < (task[1] + 1) * GPC:
                atp.step(True)
            g = proj(*task[1:])
        next(g)
        _advance(g)
        for cp in waits.get(slot, []):
            cp.wait()
        for cp in starts.get(slot, []):
            cp.start(P0)
        xrows, xdue = xready.get(slot, (xrows, xdue))
        if SCOPE and slot % SCOPE == SCOPE - 1:
            scope.close()
            scope.enter_context(jax.named_scope(f"s{slot + 1:03d}"))
        if slot >= FFN_AT and not ffn_done:
            assert route_done
            ffn_done = _advance(ffng)
        if lnp.done == lnp.n and not route_done:
            route_done = _advance(routeg)
        lcredit = min(lcredit + (xrows // 32 - lnp.started) / max(xdue - slot, 1), 1.0)
        go = lcredit >= 0.999 and lnp.started < xrows // 32
        lcredit -= go
        lnp.step(go)
        ready = sum(GPC for c in avail if avail[c] + LAG <= slot)
        rate = max([((c + 1) * GPC - atp.started) / max(need[c] - 3 - LAG - slot, 1)
                    for c in need] + [0.0])
        credit += rate
        k = 0
        while credit >= PAIR and atp.started < ready:
            credit -= PAIR
            for _ in range(PAIR):
                atp.step(True)
            k += 1
        if k == 0:
            atp.step(False)
        credit = min(credit, PAIR)
        for f in extra.get(slot, []):
            f()
    ocopy.wait()
    scope.close()


@jax.jit
def pallas_recurrent_scan__sliding_local_dilated__moe_arch_mod__prompt_kernel(
    A_x, A_wqkv, A_wo, B_x, B_w_r, B_w_gate, B_w_up, B_w_down,
):
    del B_x
    hbm = pl.BlockSpec(memory_space=pltpu.HBM)
    V = pltpu.VMEM
    out = pl.pallas_call(
        _kernel,
        in_specs=[hbm] * 7,
        out_specs=hbm,
        out_shape=jax.ShapeDtypeStruct((S, D), BF),
        scratch_shapes=[
            V((NT, S, 128), BF),
            V((4, D, D), BF),
            V((D,), BF),
            V((3, F, D), BF),
            V((4 * NT, D // 2, 128), U32),
            V((3, D // 2, D), U32),
            V((D // 2, D), U32),
            V((S // 2, D), U32),
            V((NT, S // 2, 128), U32),
            V((NT, 2, S // 2, 128), F32),
            V((NT, 2, HALO + S // 2, 128), F32),
            V((NT, 2, HALO + S // 2, 128), F32),
            V((S // 2, D), U32),
            V((S, D), BF),
            V((8, D), F32),
            pltpu.SemaphoreType.DMA((len(XCUT) - 1,)),
            pltpu.SemaphoreType.DMA((7,)),
            pltpu.SemaphoreType.DMA(()),
        ],
        compiler_params=pltpu.CompilerParams(vmem_limit_bytes=100 << 20),
        name="fused",
    )(A_x.reshape(S, D), A_wqkv, A_wo, B_w_r, B_w_gate.T, B_w_up.T, B_w_down)
    return out.reshape(1, S, D)
```

```python
import functools

import jax
import jax.numpy as jnp
import numpy as np
from jax import lax
from jax.experimental import pallas as pl
from jax.experimental.pallas import tpu as pltpu

S, D, F = 2048, 640, 1728
H, DH, W, DIL = 32, 20, 8, 2
NT = D // 128
NF = -(-F // 128)
HALO = 8
BF = jnp.bfloat16
F32 = jnp.float32
U32 = jnp.uint32
LOG2E = 1.4426950408889634
NEG = -998244352.0
EPS = 1.0013580322265625e-05


M = 128
NC = S // M
XCUT = (0, 256, 512, 1024, 2048)
FP = 1
CNT = []
EARLY = 1
REV = 6
PLAIN = 0
LITE = 1
DELAY = 0
B1 = 1
B2 = 13
B3 = 30
B4 = 50
BACK = 0
FR = 1.0
A1 = 0.8
PAIR = 2
F0 = 40
FFN_AT = 170
LN_DUE = 152
P0 = 1
PO = 1
TAIL = 3
LAG = 2
TIE = 1
SCOPE = 0


def _pack(a, b):
    return pltpu.pack_elementwise([a, b], packed_dtype=BF)


def _unpack(u):
    return [pltpu.unpack_elementwise(u, index=i, packed_dtype=BF, unpacked_dtype=F32)
            for i in range(2)]


def _rb2(a, b):
    return _unpack(_pack(a, b))


def _rb4(v):
    return _rb2(v[0], v[1]) + _rb2(v[2], v[3])


def _rb(x):
    return x.astype(BF).astype(F32)


def _nt(a, b):
    return lax.dot_general(a, b, (((1,), (1,)), ((), ())), preferred_element_type=F32)


def _nn(a, b):
    return jnp.dot(a, b, preferred_element_type=F32)


def _bf(u):
    return pltpu.bitcast(u, BF)


def _silu(x):
    h = x * 0.5
    return h * jnp.tanh(h) + h


def _sum(xs):
    return functools.reduce(jnp.add, xs)


def _advance(g):
    return next(g, "end") == "end"


class _Pipe:
    def __init__(self, make, n, last):
        self.last = last
        self.make, self.n, self.started, self.done, self.live = make, n, 0, 0, []

    def step(self, start):
        live = self.live
        self.live = []
        rest = [e for e in live if e[0] < self.last]
        for e in live:
            if e[0] == self.last:
                _advance(e[1])
                self.done += 1
        if start and self.started < self.n:
            rest.append([0, self.make(self.started)])
            self.started += 1
        for e in reversed(rest):
            next(e[1])
            e[0] += 1
        self.live = rest


class _Copies:
    def __init__(self, pairs, sem):
        self.cs = [pltpu.make_async_copy(a, b, sem) for a, b in pairs]

    def start(self, pri):
        for c in self.cs:
            c.start(priority=pri)

    def wait(self):
        if SCOPE:
            CNT.append(0)
            with jax.named_scope(f"w{len(CNT):02d}"):
                for c in self.cs:
                    c.wait()
            return
        for c in self.cs:
            c.wait()


def _kernel(x_hbm, wqkv_hbm, wo_hbm, wr_hbm, wg_hbm, wu_hbm, wd_hbm, out_hbm,
            xb, wraw, wrb, wf, stage, wt, wn, wop, xn, gate, qs, ks, vs, ob, outb, wrf,
            xsem, wsem, osem):
    col = lambda t: pl.ds(t * 128, 128)
    xu = xb.bitcast(U32)

    xcopy = [_Copies([(x_hbm.at[pl.ds(a, b - a), col(t)], xb.at[t, pl.ds(a, b - a)])
                      for t in range(NT)], xsem.at[i])
             for i, (a, b) in enumerate(zip(XCUT[:-1], XCUT[1:]))]

    def wcopy(m, a, b, sem):
        return _Copies([(wqkv_hbm.at[pl.ds(a, b - a), pl.ds(m * D, D)],
                         wraw.at[m, pl.ds(a, b - a)])], wsem.at[sem])

    kcopy = [wcopy(1, 0, 384, 0), wcopy(1, 384, D, 1)]
    vcopy = wcopy(2, 0, D, 2)
    qcopy = wcopy(0, 0, D, 3)
    wocopy = _Copies([(wo_hbm, wraw.at[3])], wsem.at[4])
    wrcopy = _Copies([(wr_hbm, wrb)], wsem.at[5])
    fcopy = _Copies([(w.at[pl.ds(j * F // FP, F // FP)], wf.at[i, pl.ds(j * F // FP, F // FP)])
                     for i, w in enumerate((wg_hbm, wu_hbm, wd_hbm)) for j in range(FP)], wsem.at[6])
    ocopy = _Copies([(outb.at[pl.ds(c * M, M), col(t)], out_hbm.at[pl.ds(c * M, M), col(t)])
                     for c in range(NC) for t in range(NT)], osem)

    if DELAY:
        pl.delay(DELAY)
    for c in (wrcopy, xcopy[0], kcopy[0], kcopy[1]) + ((xcopy[1], vcopy) if EARLY else ()):
        c.start(P0)

    def permute_rows(src, dst, t):
        for d2 in range(DH // 2):
            u = src[pl.ds(d2, H // 2, stride=DH), :]
            v = src[pl.ds(d2 + DH // 2, H // 2, stride=DH), :]
            dst[pl.ds(H * d2, H // 2), col(t)] = (u & np.uint32(0xFFFF)) | (v << 16)
            dst[pl.ds(H * d2 + H // 2, H // 2), col(t)] = (u >> 16) | (v & np.uint32(0xFFFF0000))

    def prep_a(m, kt):
        stage[m * NT + kt] = pltpu.bitcast(wraw[m, pl.ds(kt * 128, 128), :].T, U32)

    def prep_b(m, kt):
        permute_rows(stage.at[m * NT + kt], wt.at[m], kt)

    def prep_c(m, t):
        wn[m, :, col(t)] = pltpu.bitcast(_bf(after_all(wt[m, pl.ds(t * 64, 64), :])).T, U32)

    def after_all(u):
        return jnp.concatenate([jnp.concatenate([after(u[:8, t * 128:(t + 1) * 128], st["tok"][-1])
                                                 for t in range(NT)], axis=1), u[8:]], axis=0)

    def prep_wo(t):
        stage[3 * NT + t] = pltpu.bitcast(wraw[3, :, col(t)], U32)
        permute_rows(stage.at[3 * NT + t], wop, t)

    lane = lax.broadcasted_iota(jnp.int32, (8, 128), 1)
    st = {"ob": {}, "r": [jnp.zeros((8, 128), F32)] * 2}

    def after(v, dep):
        return jnp.where(st["never"], lax.bitcast_convert_type(dep, v.dtype), v)

    def mark(v):
        toks = st.setdefault("tok", [])
        v = lax.bitcast_convert_type(v, U32)
        toks.append(v ^ toks[-1] if toks else v)

    def done(v):
        st["vt"] = v ^ st["vt"] if "vt" in st else v

    def gated(u):
        hist = st.setdefault("vts", [])
        hist.append(st.get("vt"))
        if not REV or len(hist) <= REV or hist[-1 - REV] is None:
            return _bf(u)
        dep = hist[-1 - REV]
        head = jnp.concatenate([after(u[:8, t * 128:(t + 1) * 128], dep) for t in range(1)]
                               + [u[:8, 128:]], axis=1)
        return _bf(jnp.concatenate([head, u[8:]], axis=0))

    def tie(v, age=-1):
        if not TIE or "tok" not in st:
            return v
        n = v.shape[1]
        return jnp.where(st["never"][:, :n], lax.bitcast_convert_type(st["tok"][age], v.dtype)[:, :n], v)

    def ln(i):
        def load(t):
            return (_unpack(xu[t, pl.ds(16 * i, 8, stride=2), :])
                    + _unpack(xu[t, pl.ds(16 * i + 1, 8, stride=2), :]))

        x = [load(t) for t in range(NT)]
        x[0] = [tie(a) for a in x[0]]
        x = list(zip(*x))
        tot, ml, m2 = [], [], []
        for xs in x:
            s = _sum(xs)
            tot.append(jnp.sum(s, axis=1, keepdims=True))
            ml.append(s * (1.0 / NT))
            m2.append(_sum([(a - ml[-1]) * (a - ml[-1]) for a in xs]))
        yield
        mean = [jnp.broadcast_to(a, (8, 128)) * (1.0 / D) for a in tot]
        tot = [jnp.sum(b + ((a - m) * (a - m)) * float(NT), axis=1, keepdims=True)
               for a, b, m in zip(ml, m2, mean)]
        mean = [_pack(mean[0], mean[1]), _pack(mean[2], mean[3])]
        yield
        var = _rb4([jnp.broadcast_to(a, (8, 128)) * (1.0 / D) for a in tot])
        var = _rb4([a + EPS for a in var])
        if LITE:
            sd = _rb4([a * lax.rsqrt(a) for a in var])
            inv = [jnp.where(a == jnp.inf, 0.0, pltpu.reciprocal(b, full_range=False))
                   for a, b in zip(var, sd)]
        else:
            inv = [1.0 / a for a in _rb4([jnp.sqrt(a) for a in var])]
        mean = _unpack(mean[0]) + _unpack(mean[1])
        r = None
        c, j = divmod(i, M // 32)
        for t in range(NT):
            y = [a * b for a, b in zip(_rb4([a - m for a, m in zip(load(t), mean)]), inv)]
            ye, yo = _pack(y[0], y[2]), _pack(y[1], y[3])
            xn[pl.ds(c * M // 2 + 8 * j, 8), col(t)] = ye
            xn[pl.ds(c * M // 2 + M // 4 + 8 * j, 8), col(t)] = yo
            y = [b for a in zip(_unpack(ye), _unpack(yo)) for b in a]
            for h in range(2):
                a = _pack(_silu(y[2 * h]), _silu(y[2 * h + 1]))
                gate[t, pl.ds(16 * i + h, 8, stride=2), :] = a
                done(a)
            w = wrf[:, col(t)]
            a = [a * w for a in y]
            r = a if r is None else [b + e for b, e in zip(r, a)]
        r = [jnp.sum(a, axis=1, keepdims=True) for a in r]
        st["xn"] = 32 * (i + 1)
        yield
        k = i // 32
        for s in range(4):
            st["r"][k] = jnp.where(lane == (4 * i + s) % 128, r[s], st["r"][k])

    def qkv(c, m, t):
        a = gated(xn[pl.ds(c * M // 2, M // 2), :])
        if PLAIN and c >= PLAIN:
            y = _nn(a, _bf(wn[m, :, col(t)]))
        else:
            y = _nt(a, _bf(wt[m, pl.ds(t * 64, 64), :]))
        mark(y[-8:])
        yield
        for p in range(2):
            yp = y[p * M // 2:(p + 1) * M // 2]
            if m == 0:
                qs[t, p, pl.ds(c * M // 2, M // 2), :] = yp * (DH ** -0.5 * LOG2E)
            else:
                dst = ks if m == 1 else vs
                dst[t, p, pl.ds(HALO + c * M // 2, M // 2), :] = yp
                if c == 0:
                    dst[t, p, pl.ds(0, HALO), :] = jnp.broadcast_to(y[0:1, :], (HALO, 128))

    def attn(g):
        jb, par = divmod(g, 2)
        r0 = 8 * jb
        if par == 0:
            prev = st["ob"].get(jb - BACK)
            st["dep"] = [st["tok"][-1] ^ a for a in prev] if prev and BACK else [st["tok"][-1]] * NT
        q = [after(qs[t, par, pl.ds(r0, 8), :], st["dep"][t]) for t in range(NT)]
        p = []
        for w in range(W):
            rows = pl.ds(HALO + r0 - w, 8)
            p.append(_sum([q[t] * ks[t, par, rows, :] for t in range(NT)]))
        rl = [pltpu.roll(a, 64, 1) for a in p]
        yield
        p = [a + b for a, b in zip(p, rl)]
        rl = [pltpu.roll(a, 32, 1) for a in p]
        yield
        p = [a + b for a, b in zip(p, rl)]
        if jb == 0:
            row = lax.broadcasted_iota(jnp.int32, (8, 128), 0)
            p = [jnp.where(row >= w, a, NEG * LOG2E) for w, a in enumerate(p)]
        mx = functools.reduce(jnp.maximum, p)
        e = [jnp.exp2(a - mx) for a in p]
        inv = pltpu.reciprocal(_sum(e), full_range=False)
        o = [_sum([e[w] * vs[t, par, pl.ds(HALO + r0 - w, 8), :] for w in range(W)]) * inv
             for t in range(NT)]
        if par == 0:
            st["o"] = o
        else:
            st["ob"][jb] = [_pack(a, b) for a, b in zip(st["o"], o)]
            for t in range(NT):
                ob[pl.ds(r0, 8), col(t)] = st["ob"][jb][t]
                done(st["ob"][jb][t])

    def proj(c, t):
        half = pl.ds(c * M // 2, M // 2)
        s = _nn(gated(ob[half, :]), _bf(wop[:, col(t)]))
        mark(s[-8:])
        yield
        g = _bf(gate[t, half, :]).astype(F32)
        outb[pl.ds(c * M, M), col(t)] = (_bf(xu[t, half, :]).astype(F32) + s * g).astype(BF)
        ocopy.cs[c * NT + t].start(priority=PO)

    def route():
        r = jnp.concatenate(_rb2(*st["r"]), axis=1)
        key = jnp.where(r != r, -jnp.inf, r)
        slot = lax.broadcasted_iota(jnp.int32, (8, 256), 1)
        tok = (slot >> 2) * 32 + (slot & 3) + 4 * lax.broadcasted_iota(jnp.int32, (8, 256), 0)
        picks = []
        for _ in range(2):
            top = jnp.max(key, keepdims=True)
            yield
            cand = key == top
            if picks:
                cand = cand & (tok != picks[0][0])
            idx = jnp.min(jnp.where(cand, tok, S), keepdims=True)
            yield
            val = jnp.sum(jnp.where(tok == idx, r, 0.0), keepdims=True)
            picks.append((idx, val))
            key = jnp.where(tok == idx, -jnp.inf, key)
        sidx = [jnp.squeeze(i) for i, _ in picks]
        base = [pl.multiple_of((i >> 4) * 8, 8) for i in sidx]
        src = [pl.multiple_of((i >> 7) * 64 + (i & 1) * 32 + ((i >> 5) & 3) * 8, 8) for i in sidx]
        yield
        row = lax.broadcasted_iota(jnp.int32, (16, 128), 0)
        xs = []
        for t in range(NT):
            sel = [jnp.sum(jnp.where(row == ((i >> 1) & 15),
                                     _bf(xn[pl.ds(b, 8), col(t)]).astype(F32), 0.0),
                           axis=0, keepdims=True) for (i, _), b in zip(picks, src)]
            sel = [jnp.broadcast_to(a, (8, 128)) for a in sel]
            xs.append(_pack(sel[0], sel[1]))
        st["route"] = (picks, base, xs)

    def ffn():
        picks, base, xs = st["route"]
        span = lambda a, b: pl.ds(a * 128, min(b * 128, F) - a * 128)
        lhs = lambda us: jnp.concatenate([_bf(tie(u, -3)) for u in us], axis=1)
        hid = []
        for n in range(NF):
            g = _nt(lhs(xs), wf[0, span(n, n + 1), :])[:8]
            yield
            g, u = _rb2(g, _nt(lhs(xs), wf[1, span(n, n + 1), :])[:8])
            a = _rb2(_silu(g), u)[0] * u
            hid.append(_pack(a, a))
            yield
        y = None
        for n in range(NF):
            a = _nn(lhs(hid[n:n + 1]), wf[2, span(n, n + 1), :])[:8]
            y = a if y is None else y + a
            yield
        y = _rb(y)
        row = lax.broadcasted_iota(jnp.int32, (8, 128), 0)
        for j, (idx, val) in enumerate(picks):
            upd = _rb(y[2 * j:2 * j + 1] * _rb(jax.nn.sigmoid(val)))
            for t in range(NT):
                xsel = _unpack(xs[t])[j]
                g = _silu(_rb(xsel + upd[:, t * 128:(t + 1) * 128]))
                cur = _unpack(gate[t, pl.ds(base[j], 8), :])
                gate[t, pl.ds(base[j], 8), :] = _pack(
                    *[jnp.where(2 * row + p == (idx & 15), g, a) for p, a in enumerate(cur)])

    lnp = _Pipe(ln, S // 32, 3)
    atp = _Pipe(attn, S // 8, 2)
    GPC = M // 8

    wrcopy.wait()
    xcopy[0].wait()
    wrf[...] = jnp.broadcast_to(wrb[...].astype(F32).reshape(1, D), (8, D))
    st["never"] = (lax.bitcast_convert_type(wrf[:, col(0)], U32) & np.uint32(0xFFFF)) != 0
    while lnp.done < XCUT[1] // 32:
        lnp.step(lnp.started < XCUT[1] // 32)
    for cp, kts in zip(kcopy, ((0, 1, 2), (3, 4))):
        cp.wait()
        if kts[0] == 0 and not EARLY:
            xcopy[1].start(P0)
            vcopy.start(P0)
        for kt in kts:
            prep_a(1, kt)
        for kt in kts:
            prep_b(1, kt)

    tiles = lambda c, m: [("qkv", c, m, t) for t in range(NT)]
    order = [a for m in (1, 2, 0) for c in range(4) for a in tiles(c, m)]
    order += [a for c in range(4, NC) for m in (1, 2, 0) for a in tiles(c, m)]
    nffn = -(-int(44 / FR) // 5) * 5
    a = order[FFN_AT + nffn:]
    order = order[:FFN_AT + nffn]
    projs = [("proj", c, t) for c in range(NC) for t in range(NT)]
    b = projs[:-TAIL * NT]
    i = j = 0
    while i < len(a) or j < len(b):
        if j >= len(b) or (i < len(a) and i * len(b) < j * len(a)):
            order += a[i:i + NT]
            i += NT
        else:
            order += b[j:j + NT]
            j += NT
    order += projs[-TAIL * NT:]

    need = {t[1]: s for s, t in enumerate(order) if t[0] == "proj" and t[2] == 0}
    avail = {t[1]: s for s, t in enumerate(order) if t[0] == "qkv" and t[2:] == (0, NT - 1)}

    P = functools.partial
    waits = {B1: [xcopy[1]], B2: [vcopy], B3: [qcopy, xcopy[2]], B4: [xcopy[3]],
             FFN_AT: [wocopy, fcopy]}
    starts = {B1: [qcopy, xcopy[2]], B2: [xcopy[3]], F0: [wocopy, fcopy]}
    xready = {B1: (XCUT[2], B2 - 2), B3: (XCUT[3], 75), B4: (XCUT[4], LN_DUE)}
    extra = {}
    for kt in range(NT):
        extra.setdefault(B2 + kt, []).append(P(prep_a, 2, kt))
        extra.setdefault(B2 + 1 + kt, []).append(P(prep_b, 2, kt))
        extra.setdefault(B3 + kt, []).append(P(prep_a, 0, kt))
        extra.setdefault(B3 + 2 + kt, []).append(P(prep_b, 0, kt))
        extra.setdefault(FFN_AT + 5 * kt, []).append(P(prep_wo, kt))
        if PLAIN:
            extra.setdefault(20 + kt, []).append(P(prep_c, 1, kt))
            extra.setdefault(25 + kt, []).append(P(prep_c, 2, kt))
            extra.setdefault(B3 + 9 + kt, []).append(P(prep_c, 0, kt))

    routeg, ffng = route(), ffn()
    route_done = ffn_done = False
    xrows, xdue, lcredit = XCUT[1], 0, 0.0
    credit = fcredit = 0.0
    for slot, task in enumerate(order):
        if task[0] == "qkv":
            while st["xn"] < (task[1] + 1) * M:
                lnp.step(lnp.started < xrows // 32)
            g = qkv(*task[1:])
        else:
            while not ffn_done:
                ffn_done = _advance(ffng)
            while atp.done < (task[1] + 1) * GPC:
                atp.step(True)
            g = proj(*task[1:])
        next(g)
        _advance(g)
        for cp in waits.get(slot, []):
            cp.wait()
        for cp in starts.get(slot, []):
            cp.start(P0)
        xrows, xdue = xready.get(slot, (xrows, xdue))
        if slot >= FFN_AT and not ffn_done:
            assert route_done
            fcredit += FR
            if fcredit >= 1:
                fcredit -= 1
                ffn_done = _advance(ffng)
        if lnp.done == lnp.n and not route_done:
            route_done = _advance(routeg)
        lcredit = min(lcredit + (xrows // 32 - lnp.started) / max(xdue - slot, 1), 1.0)
        go = lcredit >= 0.999 and lnp.started < xrows // 32
        lcredit -= go
        lnp.step(go)
        ready = sum(GPC for c in avail if avail[c] + LAG <= slot)
        rate = max([((c + 1) * GPC - atp.started) / max(need[c] - 3 - LAG - slot, 1)
                    for c in need] + [0.0])
        credit += rate if slot > LN_DUE else min(rate, A1)
        k = 0
        while credit >= PAIR and atp.started < ready:
            credit -= PAIR
            for _ in range(PAIR):
                atp.step(True)
            k += 1
        if k == 0:
            atp.step(False)
        credit = min(credit, PAIR)
        for f in extra.get(slot, []):
            f()
    ocopy.wait()


@jax.jit
def pallas_recurrent_scan__sliding_local_dilated__moe_arch_mod__prompt_kernel(
    A_x, A_wqkv, A_wo, B_x, B_w_r, B_w_gate, B_w_up, B_w_down,
):
    del B_x
    hbm = pl.BlockSpec(memory_space=pltpu.HBM)
    V = pltpu.VMEM
    out = pl.pallas_call(
        _kernel,
        in_specs=[hbm] * 7,
        out_specs=hbm,
        out_shape=jax.ShapeDtypeStruct((S, D), BF),
        scratch_shapes=[
            V((NT, S, 128), BF),
            V((4, D, D), BF),
            V((D,), BF),
            V((3, F, D), BF),
            V((4 * NT, D // 2, 128), U32),
            V((3, D // 2, D), U32),
            V((3, D // 2, D), U32),
            V((D // 2, D), U32),
            V((S // 2, D), U32),
            V((NT, S // 2, 128), U32),
            V((NT, 2, S // 2, 128), F32),
            V((NT, 2, HALO + S // 2, 128), F32),
            V((NT, 2, HALO + S // 2, 128), F32),
            V((S // 2, D), U32),
            V((S, D), BF),
            V((8, D), F32),
            pltpu.SemaphoreType.DMA((len(XCUT) - 1,)),
            pltpu.SemaphoreType.DMA((7,)),
            pltpu.SemaphoreType.DMA(()),
        ],
        compiler_params=pltpu.CompilerParams(vmem_limit_bytes=100 << 20),
        name="fused",
    )(A_x.reshape(S, D), A_wqkv, A_wo, B_w_r, B_w_gate.T, B_w_up.T, B_w_down)
    return out.reshape(1, S, D)
```

```python
import functools

import jax
import jax.numpy as jnp
import numpy as np
from jax import lax
from jax.experimental import pallas as pl
from jax.experimental.pallas import tpu as pltpu


S, D, F = 2048, 640, 1728
H, DH, W = 32, 20, 8
NT = D // 128
NF = -(-F // 128)
HALO = 8
BF, F32, U32, I32 = jnp.bfloat16, jnp.float32, jnp.uint32, jnp.int32
LOG2E = 1.4426950408889634
NEG = -998244352.0
EPS = 1.0013580322265625e-05

M = 128
NC = S // M
NK = 6
XCUT = (0, 128, 384, NK * M, S)
KCUT = (0, 384, D)
B1 = 6
B2 = 21
B3 = 50
F0 = 40
FFN_AT = 172
FFN_LEN = 60
LN0_DUE = 4
LN1_DUE = 18
LN2_DUE = 150
TAIL = 3
LAG = 2
REV = 7
BACK = 3
PAIR = 1
A1 = 0.5
PK = 0
RND = 1
P0 = 1
DELAY = 0
SCOPE = 0


def _pack(a, b):
    return pltpu.pack_elementwise([a, b], packed_dtype=BF)


def _unpack(u):
    return [pltpu.unpack_elementwise(u, index=i, packed_dtype=BF, unpacked_dtype=F32)
            for i in range(2)]


def _round2(a, b):
    return _unpack(_pack(a, b))


def _round4(v):
    return _round2(v[0], v[1]) + _round2(v[2], v[3])


def _round(x):
    return x.astype(BF).astype(F32)


def _nt(a, b):
    return lax.dot_general(a, b, (((1,), (1,)), ((), ())), preferred_element_type=F32)


def _nn(a, b):
    return jnp.dot(a, b, preferred_element_type=F32)


def _bf(u):
    return pltpu.bitcast(u, BF)


def _silu(x, half=0.5):
    h = x * half
    return h * jnp.tanh(h) + h


def _sum(xs):
    return functools.reduce(jnp.add, xs)


def _col(t, n=1):
    return pl.ds(t * 128, n * 128)


def _advance(g):
    return next(g, "end") == "end"


class _Copies:
    def __init__(self, pairs, sem, pri=P0):
        self.pri = pri
        self.cs = [pltpu.make_async_copy(a, b, sem) for a, b in pairs]

    def start(self):
        for c in self.cs:
            c.start(priority=self.pri)

    def wait(self):
        for c in self.cs:
            c.wait()


def _slot_order():
    tiles = lambda c, m: [("qkv", c, m, t) for t in range(NT)]
    order = [a for m in (1, 2, 0) for c in range(NK) for a in tiles(c, m)]
    order += [a for c in range(NK, NC) for m in (1, 2, 0) for a in tiles(c, m)]
    order, a = order[:FFN_AT + FFN_LEN], order[FFN_AT + FFN_LEN:]
    projs = [("proj", c, t) for c in range(NC) for t in range(NT)]
    b = projs[:-TAIL * NT]
    i = j = 0
    while i < len(a) or j < len(b):
        if j >= len(b) or (i < len(a) and i * len(b) < j * len(a)):
            order += a[i:i + NT]
            i += NT
        else:
            order += b[j:j + NT]
            j += NT
    return order + projs[-TAIL * NT:]


def _kernel(x_hbm, wqkv_hbm, wo_hbm, wr_hbm, wg_hbm, wu_hbm, wd_hbm, out_hbm,
            xb, wraw, wrb, wrf, wf, stage, wt, wop, xn, gate, qs, ks, vs, ob, outb,
            wsem, osem):
    xu = xb.bitcast(U32)
    xcopy = [_Copies([(x_hbm.at[pl.ds(a, b - a), _col(t)], xb.at[t, pl.ds(a, b - a)])
                      for t in range(NT)], wsem.at[6 + i])
             for i, (a, b) in enumerate(zip(XCUT[:-1], XCUT[1:]))]

    def wcopy(m, a, b, sem):
        return _Copies([(wqkv_hbm.at[pl.ds(a, b - a), _col(m * NT, NT)],
                         wraw.at[m, pl.ds(a, b - a)])], wsem.at[sem])

    kcopy = [wcopy(1, KCUT[0], KCUT[1], 0), wcopy(1, KCUT[1], KCUT[2], 1)]
    vcopy = wcopy(2, 0, D, 2)
    qcopy = wcopy(0, 0, D, 3)
    wrcopy = _Copies([(wr_hbm, wrb)], wsem.at[4])
    fcopy = _Copies([(wo_hbm, wraw.at[3]), (wg_hbm, wf.at[0]), (wu_hbm, wf.at[1]),
                     (wd_hbm, wf.at[2])], wsem.at[5], 1)

    lane = lax.broadcasted_iota(I32, (8, 128), 1)
    st = {"r": [jnp.zeros((8, 128), F32)] * 2, "xn": 0, "gated": 0,
          "mxu": [], "vpu": None, "hist": [], "ob": {}}

    def wait(cp):
        if SCOPE:
            st["nw"] = st.get("nw", 0) + 1
            with jax.named_scope(f"w{st['nw']:02d}"):
                cp.wait()
        else:
            cp.wait()

    def after(v, dep):
        n = v.shape[1]
        return jnp.where(st["never"][:, :n], lax.bitcast_convert_type(dep, v.dtype)[:, :n], v)

    def mxu_done(v):
        v = lax.bitcast_convert_type(v, U32)
        st["mxu"].append(v ^ st["mxu"][-1] if st["mxu"] else v)

    def vpu_done(v):
        st["vpu"] = v if st["vpu"] is None else v ^ st["vpu"]

    def paced(v, age=-1):
        return after(v, st["mxu"][age]) if st["mxu"] else v

    def gated(u):
        st["hist"].append(st["vpu"])
        if len(st["hist"]) <= REV:
            return u
        head = jnp.concatenate([after(u[:8, :128], st["hist"][-1 - REV]), u[:8, 128:]], axis=1)
        return jnp.concatenate([head, u[8:]], axis=0)

    def permute_rows(src, dst, t):
        for d2 in range(DH // 2):
            u = src[pl.ds(d2, H // 2, stride=DH), :]
            v = src[pl.ds(d2 + DH // 2, H // 2, stride=DH), :]
            dst[pl.ds(H * d2, H // 2), _col(t)] = (u & np.uint32(0xFFFF)) | (v << 16)
            dst[pl.ds(H * d2 + H // 2, H // 2), _col(t)] = (u >> 16) | (v & np.uint32(0xFFFF0000))

    def prep_a(m, t):
        stage[m * NT + t] = pltpu.bitcast(wraw[m, _col(t), :].T, U32)

    def prep_b(m, t):
        permute_rows(stage.at[m * NT + t], wt.at[m], t)

    def prep_wo(t):
        stage[3 * NT + t] = pltpu.bitcast(wraw[3, :, _col(t)], U32)
        permute_rows(stage.at[3 * NT + t], wop, t)

    def xn_rows(i, par):
        c, j = divmod(i, M // 32)
        return pl.ds(c * M // 2 + par * M // 4 + 8 * j, 8)

    def norm(i):
        def load(t):
            return (_unpack(xu[t, pl.ds(16 * i, 8, stride=2), :])
                    + _unpack(xu[t, pl.ds(16 * i + 1, 8, stride=2), :]))

        x = [load(t) for t in range(NT)]
        x[0] = [paced(a) for a in x[0]]
        tot, ml, m2 = [], [], []
        for xs in zip(*x):
            s = _sum(xs)
            tot.append(jnp.sum(s, axis=1, keepdims=True))
            ml.append(s * (1.0 / NT))
            m2.append(_sum([(a - ml[-1]) * (a - ml[-1]) for a in xs]))
        yield
        mean = [jnp.broadcast_to(a, (8, 128)) * (1.0 / D) for a in tot]
        tot = [jnp.sum(b + ((a - m) * (a - m)) * float(NT), axis=1, keepdims=True)
               for a, b, m in zip(ml, m2, mean)]
        mean = [_pack(mean[0], mean[1]), _pack(mean[2], mean[3])]
        yield
        var = _round4([jnp.broadcast_to(a, (8, 128)) * (1.0 / D) for a in tot])
        var = _round4([a + EPS for a in var])
        sd = _round4([a * lax.rsqrt(a) for a in var])
        inv = [jnp.where(a == jnp.inf, 0.0, pltpu.reciprocal(b, full_range=False))
               for a, b in zip(var, sd)]
        mean = _unpack(mean[0]) + _unpack(mean[1])
        r = None
        for t in range(NT):
            y = [a - m for a, m in zip(load(t), mean)]
            y = [a * b for a, b in zip(_round4(y) if RND else y, inv)]
            ye, yo = _pack(y[0], y[2]), _pack(y[1], y[3])
            xn[xn_rows(i, 0), _col(t)] = ye
            xn[xn_rows(i, 1), _col(t)] = yo
            if RND:
                y = [b for a in zip(_unpack(ye), _unpack(yo)) for b in a]
            a = [a * wrf[:, _col(t)] for a in y]
            r = a if r is None else [b + e for b, e in zip(r, a)]
        vpu_done(ye ^ yo)
        r = [jnp.sum(a, axis=1, keepdims=True) for a in r]
        st["xn"] = 32 * (i + 1)
        yield
        for s in range(4):
            st["r"][i // 32] = jnp.where(lane == (4 * i + s) % 128, r[s], st["r"][i // 32])
        vpu_done(lax.bitcast_convert_type(st["r"][i // 32], U32))

    def gating(i):
        half = paced(jnp.full((8, 128), 0.5, F32))
        for t in range(NT):
            e, o = [_unpack(xn[xn_rows(i, p), _col(t)]) for p in range(2)]
            for h in range(2):
                a = _pack(_silu(e[h], half), _silu(o[h], half))
                gate[t, pl.ds(16 * i + h, 8, stride=2), :] = a
        vpu_done(a)

    def product(task, k0, k1):
        half, k = pl.ds(task[1] * M // 2, M // 2), _col(k0, k1 - k0)
        wrap = gated if k0 == 0 else (lambda u: u)
        if task[0] == "qkv":
            return _nt(_bf(wrap(xn[half, k])), _bf(wt[task[2], pl.ds(task[3] * 64, 64), k]))
        return _nn(_bf(wrap(ob[half, k])), _bf(wop[pl.ds(k0 * 64, (k1 - k0) * 64), _col(task[2])]))

    def store_qkv(y, c, m, t):
        dst, off = ((qs, 0), (ks, HALO), (vs, HALO))[m]
        for p in range(2):
            dst[t, p, pl.ds(off + c * M // 2, M // 2), :] = y[p * M // 2:(p + 1) * M // 2]
            if off and c == 0:
                dst[t, p, pl.ds(0, HALO), :] = jnp.broadcast_to(y[0:1, :], (HALO, 128))

    def store_out(s, c, t):
        half, rows = pl.ds(c * M // 2, M // 2), pl.ds(c * M, M)
        g = _bf(gate[t, half, :]).astype(F32)
        outb[rows, _col(t)] = (_bf(xu[t, half, :]).astype(F32) + s * g).astype(BF)
        pltpu.make_async_copy(outb.at[rows, _col(t)], out_hbm.at[rows, _col(t)], osem).start(
            priority=1)

    def attend(jb):
        r0 = 8 * jb
        dep = st["mxu"][-1]
        for a in (st["ob"].get(jb - BACK, []) if BACK else []):
            dep = dep ^ a
        scale = after(jnp.full((8, 128), DH ** -0.5 * LOG2E, F32), dep)
        win = [pl.ds(HALO + r0 - w, 8) for w in range(W)]

        def logits(par):
            q = [qs[t, par, pl.ds(r0, 8), :] * scale for t in range(NT)]
            return [_sum([q[t] * ks[t, par, r, :] for t in range(NT)]) for r in win]

        def weights(p):
            if jb == 0:
                row = lax.broadcasted_iota(I32, (8, 128), 0)
                p = [jnp.where(row >= w, a, NEG * LOG2E) for w, a in enumerate(p)]
            mx = functools.reduce(jnp.maximum, p)
            e = [jnp.exp2(a - mx) for a in p]
            return e, pltpu.reciprocal(_sum(e), full_range=False)

        def mix(par, e):
            return [_sum([a * vs[t, par, r, :] for a, r in zip(e, win)]) for t in range(NT)]

        if PK:
            ev = (lane & 32) == 0
            p = [jnp.where(ev, a, b) + pltpu.roll(jnp.where(ev, b, a), 32, 1)
                 for a, b in zip(logits(0), logits(1))]
            e, inv = weights([a + pltpu.roll(a, 64, 1) for a in p])
            e = [a * inv for a in e]
            r = [pltpu.roll(a, 32, 1) for a in e]
            o = [mix(0, [jnp.where(ev, a, b) for a, b in zip(e, r)]),
                 mix(1, [jnp.where(ev, b, a) for a, b in zip(e, r)])]
        else:
            o = []
            for par in range(2):
                p = [a + pltpu.roll(a, 64, 1) for a in logits(par)]
                e, inv = weights([a + pltpu.roll(a, 32, 1) for a in p])
                o.append([a * inv for a in mix(par, e)])
        st["ob"][jb] = [_pack(a, b) for a, b in zip(*o)]
        for t in range(NT):
            ob[pl.ds(r0, 8), _col(t)] = st["ob"][jb][t]
        vpu_done(st["ob"][jb][-1])

    def route():
        r = jnp.concatenate(_round2(*st["r"]), axis=1)
        key = jnp.where(r != r, -jnp.inf, r)
        slot = lax.broadcasted_iota(I32, (8, 256), 1)
        tok = (slot >> 2) * 32 + (slot & 3) + 4 * lax.broadcasted_iota(I32, (8, 256), 0)
        tok = tok.astype(F32)
        both = lambda f, a: f(f(a, axis=0, keepdims=True), axis=1, keepdims=True)
        full = lambda a: lax.bitcast_convert_type(jnp.broadcast_to(a, (8, 128)), U32)
        picks = []
        for _ in range(2):
            top = both(jnp.max, key)
            yield
            cand = key == top
            if picks:
                cand = cand & (tok != picks[0][0])
            idx = both(jnp.min, jnp.where(cand, tok, float(S)))
            yield
            vpu_done(full(idx))
            picks.append((idx, both(jnp.sum, jnp.where(tok == idx, r, 0.0))))
            key = jnp.where(tok == idx, -jnp.inf, key)
        picks = [(i.astype(I32), a) for i, a in picks]
        sidx = [jnp.squeeze(i) for i, _ in picks]
        base = [pl.multiple_of((i >> 4) * 8, 8) for i in sidx]
        src = [pl.multiple_of((i >> 7) * 64 + (i & 1) * 32 + ((i >> 5) & 3) * 8, 8) for i in sidx]
        yield
        row = lax.broadcasted_iota(I32, (16, 128), 0)
        xs = []
        for t in range(NT):
            sel = [jnp.sum(jnp.where(row == ((i >> 1) & 15),
                                     _bf(xn[pl.ds(b, 8), _col(t)]).astype(F32), 0.0),
                           axis=0, keepdims=True) for (i, _), b in zip(picks, src)]
            xs.append(_pack(*[jnp.broadcast_to(a, (8, 128)) for a in sel]))
        for a in xs + [full(a) for _, a in picks]:
            vpu_done(a)
        st["route"] = (picks, base, xs)

    def ffn():
        picks, base, xs = st["route"]
        span = lambda a, b: pl.ds(a * 128, min(b * 128, F) - a * 128)
        lhs = lambda us: jnp.concatenate([_bf(paced(u, -3)) for u in us], axis=1)
        hid = []
        for n0 in range(0, NF, 2):
            rem = {(i, n): _nt(lhs(xs[4:]), wf[i, span(n, n + 1), _col(4)])[:8]
                   for n in (n0, n0 + 1) for i in range(2)}
            yield
            for n in (n0, n0 + 1):
                gu = []
                for i in range(2):
                    gu.append(_nt(lhs(xs[:4]), wf[i, span(n, n + 1), _col(0, 4)])[:8] + rem[i, n])
                    yield
                g, u = _round2(*gu)
                a = _round2(_silu(g), u)[0] * u
                hid.append(_pack(a, a))
        y = y4 = None
        for n in range(NF):
            a = _nn(lhs(hid[n:n + 1]), wf[2, span(n, n + 1), _col(0, 4)])[:8]
            y = a if y is None else y + a
            yield
        for n0 in range(0, NF, 4):
            a = _nn(lhs(hid[n0:n0 + 4]), wf[2, span(n0, min(n0 + 4, NF)), _col(4)])[:8]
            y4 = a if y4 is None else y4 + a
            yield
        y = _round(jnp.concatenate([y, y4], axis=1))
        assert st["gated"] == S // 32
        row = lax.broadcasted_iota(I32, (8, 128), 0)
        for j, (idx, val) in enumerate(picks):
            upd = _round(y[2 * j:2 * j + 1] * _round(jax.nn.sigmoid(val)))
            for t in range(NT):
                g = _silu(_round(_unpack(xs[t])[j] + upd[:, t * 128:(t + 1) * 128]))
                cur = _unpack(gate[t, pl.ds(base[j], 8), :])
                gate[t, pl.ds(base[j], 8), :] = _pack(
                    *[jnp.where(2 * row + p == (idx & 15), g, a) for p, a in enumerate(cur)])

    for cp in (wrcopy, xcopy[0], kcopy[0], kcopy[1], xcopy[1], xcopy[2], vcopy):
        cp.start()
    wait(xcopy[0])
    wait(wrcopy)
    wrf[...] = jnp.broadcast_to(wrb[...].astype(F32).reshape(1, D), (8, D))
    st["never"] = (lax.bitcast_convert_type(wrf[:, _col(0)], I32) & 0xFFFF) != 0
    started = XCUT[1] // 32
    live = [norm(i) for i in range(started)]
    while live:
        live = [g for g in live if not _advance(g)]
    for cp, a, b in zip(kcopy, KCUT[:-1], KCUT[1:]):
        wait(cp)
        for f in (prep_a, prep_b):
            for t in range(a // 128, b // 128):
                f(1, t)
    wait(xcopy[1])
    live = [norm(started + i) for i in range(M // 32)]
    started += M // 32
    live = [g for g in live if not _advance(g)]

    order = _slot_order()
    app = M // 16
    need = {t[1]: s - s % 4 for s, t in enumerate(order) if t[0] == "proj" and t[2] == 0}
    avail = {t[1]: s for s, t in enumerate(order) if t[0] == "qkv" and t[2:] == (0, NT - 1)}
    waits = {B1: [xcopy[2]], B2: [vcopy], B3: [xcopy[3], qcopy], FFN_AT: [fcopy]}
    starts = {B1: [xcopy[3], qcopy], F0: [fcopy]}
    arrived = {B1: (XCUT[3], LN1_DUE), B3: (XCUT[4], LN2_DUE)}
    extra = {}
    for t in range(NT):
        for s, f, args in ((B2 + t, prep_a, (2, t)), (B2 + 1 + t, prep_b, (2, t)),
                           (B3 + t, prep_a, (0, t)), (B3 + 2 + t, prep_b, (0, t)),
                           (FFN_AT + 5 * t, prep_wo, (t,))):
            extra.setdefault(s, []).append(functools.partial(f, *args))

    routeg, ffng = route(), ffn()
    route_done = ffn_done = False
    xrows, xdue = XCUT[2], LN0_DUE
    attended = 0
    lcredit = gcredit = acredit = 0.0
    for slot, task in enumerate(order):
        if slot % 4 == 0:
            for u in order[slot:slot + 4]:
                assert (st["xn"] >= (u[1] + 1) * M if u[0] == "qkv"
                        else attended >= (u[1] + 1) * app), (slot, u)
            rem = [product(u, 4, NT) for u in order[slot:slot + 4]]
        y = product(task, 0, 4) + rem[slot % 4]
        mxu_done(y[-8:])
        if task[0] == "qkv":
            store_qkv(y, *task[1:])
        else:
            assert ffn_done
            store_out(y, *task[1:])
        for cp in waits.get(slot, []):
            wait(cp)
        for cp in starts.get(slot, []):
            cp.start()
        xrows, xdue = arrived.get(slot, (xrows, xdue))

        if slot >= FFN_AT and not ffn_done:
            assert route_done
            ffn_done = _advance(ffng)
        if started == S // 32 and not live and not route_done:
            route_done = _advance(routeg)
        lcredit = min(lcredit + (xrows // 32 - started) / max(xdue - slot, 1), 1.0)
        if lcredit >= 0.999 and started < xrows // 32:
            lcredit -= 1
            live.append(norm(started))
            started += 1
        live = [g for g in live if not _advance(g)]

        for lim, s0, s1 in ((XCUT[3] // 32, NT * NK, B3),
                            (S // 32, LN2_DUE + 2, FFN_AT + FFN_LEN - 10)):
            if s0 <= slot and st["gated"] < lim:
                gcredit += (lim - st["gated"]) / max(s1 - slot, 1)
                while gcredit >= 0.999 and st["gated"] < lim:
                    gcredit -= 1
                    gating(st["gated"])
                    st["gated"] += 1
                break

        ready = sum(app for c in avail if avail[c] + LAG <= slot)
        rate = max((c + 1) * app - attended for c in need) and max(
            ((c + 1) * app - attended) / max(need[c] - 3 - LAG - slot, 1) for c in need)
        acredit += rate if slot > LN2_DUE else min(rate, A1)
        while acredit >= PAIR and attended < ready:
            acredit -= PAIR
            for _ in range(PAIR):
                attend(attended)
                attended += 1
        acredit = min(acredit, PAIR)
        for f in extra.get(slot, []):
            f()
    pltpu.make_async_copy(outb, out_hbm, osem).wait()


@jax.jit
def pallas_recurrent_scan__sliding_local_dilated__moe_arch_mod__prompt_kernel(
    A_x, A_wqkv, A_wo, B_x, B_w_r, B_w_gate, B_w_up, B_w_down,
):
    del B_x
    hbm = pl.BlockSpec(memory_space=pltpu.HBM)
    V = pltpu.VMEM
    out = pl.pallas_call(
        _kernel,
        in_specs=[hbm] * 7,
        out_specs=hbm,
        out_shape=jax.ShapeDtypeStruct((S, D), BF),
        scratch_shapes=[
            V((NT, S, 128), BF),
            V((4, D, D), BF),
            V((D,), BF),
            V((8, D), F32),
            V((3, F, D), BF),
            V((4 * NT, D // 2, 128), U32),
            V((3, D // 2, D), U32),
            V((D // 2, D), U32),
            V((S // 2, D), U32),
            V((NT, S // 2, 128), U32),
            V((NT, 2, S // 2, 128), F32),
            V((NT, 2, HALO + S // 2, 128), F32),
            V((NT, 2, HALO + S // 2, 128), F32),
            V((S // 2, D), U32),
            V((S, D), BF),
            pltpu.SemaphoreType.DMA((5 + len(XCUT),)),
            pltpu.SemaphoreType.DMA(()),
        ],
        compiler_params=pltpu.CompilerParams(vmem_limit_bytes=100 << 20),
        name="fused",
    )(A_x.reshape(S, D), A_wqkv, A_wo, B_w_r, B_w_gate.T, B_w_up.T, B_w_down)
    return out.reshape(1, S, D)
```

```python
import functools

import jax
import jax.numpy as jnp
import numpy as np
from jax import lax
from jax.experimental import pallas as pl
from jax.experimental.pallas import tpu as pltpu


S, D, F = 2048, 640, 1728
H, DH, W = 32, 20, 8
NT = D // 128
NF = -(-F // 128)
HALO = 8
BF, F32, U32, I32 = jnp.bfloat16, jnp.float32, jnp.uint32, jnp.int32
LOG2E = 1.4426950408889634
NEG = -998244352.0
EPS = 1.0013580322265625e-05

M = 128
NC = S // M
NK = 6
XCUT = (0, 128, 384, NK * M, S)
KCUT = (0, 384, D)
B1 = 6
B2 = 21
B3 = 50
F0 = 40
FFN_AT = 180
FFN_LEN = 60
LN0_DUE = 4
LN1_DUE = 18
LN2_DUE = 156
TAIL = 3
LAG = 2
REV = 7
BACK = 3
PAIR = 1
A1 = 0.43
PK = 0
RND = 1
P0 = 1
DELAY = 0
RS = 3
G0 = 170
STAG = 0
EPI = 0
SCOPE = 0


def _pack(a, b):
    return pltpu.pack_elementwise([a, b], packed_dtype=BF)


def _unpack(u):
    return [pltpu.unpack_elementwise(u, index=i, packed_dtype=BF, unpacked_dtype=F32)
            for i in range(2)]


def _round2(a, b):
    return _unpack(_pack(a, b))


def _round4(v):
    return _round2(v[0], v[1]) + _round2(v[2], v[3])


def _round(x):
    return x.astype(BF).astype(F32)


def _nt(a, b):
    return lax.dot_general(a, b, (((1,), (1,)), ((), ())), preferred_element_type=F32)


def _nn(a, b):
    return jnp.dot(a, b, preferred_element_type=F32)


def _bf(u):
    return pltpu.bitcast(u, BF)


def _silu(x, half=0.5):
    h = x * half
    return h * jnp.tanh(h) + h


def _sum(xs):
    return functools.reduce(jnp.add, xs)


def _col(t, n=1):
    return pl.ds(t * 128, n * 128)


def _advance(g):
    return next(g, "end") == "end"


class _Copies:
    def __init__(self, pairs, sem, pri=P0):
        self.pri = pri
        self.cs = [pltpu.make_async_copy(a, b, sem) for a, b in pairs]

    def start(self):
        for c in self.cs:
            c.start(priority=self.pri)

    def wait(self):
        for c in self.cs:
            c.wait()


def _slot_order():
    tiles = lambda c, m: [("qkv", c, m, t) for t in range(NT)]
    order = [a for m in (1, 2, 0) for c in range(NK) for a in tiles(c, m)]
    order += [a for c in range(NK, NC) for m in (1, 2, 0) for a in tiles(c, m)]
    order, a = order[:FFN_AT + FFN_LEN], order[FFN_AT + FFN_LEN:]
    projs = [("proj", c, t) for c in range(NC) for t in range(NT)]
    b = projs[:-TAIL * NT]
    i = j = 0
    while i < len(a) or j < len(b):
        if j >= len(b) or (i < len(a) and i * len(b) < j * len(a)):
            order += a[i:i + NT]
            i += NT
        else:
            order += b[j:j + NT]
            j += NT
    return order + projs[-TAIL * NT:]


def _kernel(x_hbm, wqkv_hbm, wo_hbm, wr_hbm, wg_hbm, wu_hbm, wd_hbm, out_hbm,
            xb, wraw, wrb, wrf, wf, stage, wt, wop, xn, gate, qs, ks, vs, ob, outb,
            wsem, osem):
    xu = xb.bitcast(U32)
    xcopy = [_Copies([(x_hbm.at[pl.ds(a, b - a), _col(t)], xb.at[t, pl.ds(a, b - a)])
                      for t in range(NT)], wsem.at[6 + i])
             for i, (a, b) in enumerate(zip(XCUT[:-1], XCUT[1:]))]

    def wcopy(m, a, b, sem):
        return _Copies([(wqkv_hbm.at[pl.ds(a, b - a), _col(m * NT, NT)],
                         wraw.at[m, pl.ds(a, b - a)])], wsem.at[sem])

    kcopy = [wcopy(1, KCUT[0], KCUT[1], 0), wcopy(1, KCUT[1], KCUT[2], 1)]
    vcopy = wcopy(2, 0, D, 2)
    qcopy = wcopy(0, 0, D, 3)
    wrcopy = _Copies([(wr_hbm, wrb)], wsem.at[4])
    fcopy = _Copies([(wo_hbm, wraw.at[3]), (wg_hbm, wf.at[0]), (wu_hbm, wf.at[1]),
                     (wd_hbm, wf.at[2])], wsem.at[5], 1)

    lane = lax.broadcasted_iota(I32, (8, 128), 1)
    st = {"r": [jnp.zeros((8, 128), F32)] * 2, "xn": 0, "gated": 0,
          "mxu": [], "vpu": None, "hist": [], "ob": {}}

    def wait(cp):
        if SCOPE:
            st["nw"] = st.get("nw", 0) + 1
            with jax.named_scope(f"w{st['nw']:02d}"):
                cp.wait()
        else:
            cp.wait()

    def after(v, dep):
        n = v.shape[1]
        return jnp.where(st["never"][:, :n], lax.bitcast_convert_type(dep, v.dtype)[:, :n], v)

    def mxu_done(v):
        v = lax.bitcast_convert_type(v, U32)
        st["mxu"].append(v ^ st["mxu"][-1] if st["mxu"] else v)

    def vpu_done(v):
        st["vpu"] = v if st["vpu"] is None else v ^ st["vpu"]

    def paced(v, age=-1):
        return after(v, st["mxu"][age]) if st["mxu"] else v

    def gated(u):
        st["hist"].append(st["vpu"])
        if len(st["hist"]) <= REV:
            return u
        head = jnp.concatenate([after(u[:8, :128], st["hist"][-1 - REV]), u[:8, 128:]], axis=1)
        return jnp.concatenate([head, u[8:]], axis=0)

    def permute_rows(src, dst, t):
        for d2 in range(DH // 2):
            u = src[pl.ds(d2, H // 2, stride=DH), :]
            v = src[pl.ds(d2 + DH // 2, H // 2, stride=DH), :]
            dst[pl.ds(H * d2, H // 2), _col(t)] = (u & np.uint32(0xFFFF)) | (v << 16)
            dst[pl.ds(H * d2 + H // 2, H // 2), _col(t)] = (u >> 16) | (v & np.uint32(0xFFFF0000))

    def prep_a(m, t):
        stage[m * NT + t] = pltpu.bitcast(wraw[m, _col(t), :].T, U32)

    def prep_b(m, t):
        permute_rows(stage.at[m * NT + t], wt.at[m], t)

    def prep_wo(t):
        stage[3 * NT + t] = pltpu.bitcast(wraw[3, :, _col(t)], U32)
        permute_rows(stage.at[3 * NT + t], wop, t)

    def xn_rows(i, par):
        c, j = divmod(i, M // 32)
        return pl.ds(c * M // 2 + par * M // 4 + 8 * j, 8)

    def norm(i):
        def load(t):
            return (_unpack(xu[t, pl.ds(16 * i, 8, stride=2), :])
                    + _unpack(xu[t, pl.ds(16 * i + 1, 8, stride=2), :]))

        x = [load(t) for t in range(NT)]
        x[0] = [paced(a) for a in x[0]]
        tot, ml, m2 = [], [], []
        for xs in zip(*x):
            s = _sum(xs)
            tot.append(jnp.sum(s, axis=1, keepdims=True))
            ml.append(s * (1.0 / NT))
            m2.append(_sum([(a - ml[-1]) * (a - ml[-1]) for a in xs]))
        yield
        mean = [jnp.broadcast_to(a, (8, 128)) * (1.0 / D) for a in tot]
        tot = [jnp.sum(b + ((a - m) * (a - m)) * float(NT), axis=1, keepdims=True)
               for a, b, m in zip(ml, m2, mean)]
        mean = [_pack(mean[0], mean[1]), _pack(mean[2], mean[3])]
        yield
        var = _round4([jnp.broadcast_to(a, (8, 128)) * (1.0 / D) for a in tot])
        var = _round4([a + EPS for a in var])
        sd = _round4([a * lax.rsqrt(a) for a in var])
        inv = [jnp.where(a == jnp.inf, 0.0, pltpu.reciprocal(b, full_range=False))
               for a, b in zip(var, sd)]
        mean = _unpack(mean[0]) + _unpack(mean[1])
        r = None
        for t in range(NT):
            y = [a - m for a, m in zip(load(t), mean)]
            y = [a * b for a, b in zip(_round4(y) if RND else y, inv)]
            ye, yo = _pack(y[0], y[2]), _pack(y[1], y[3])
            xn[xn_rows(i, 0), _col(t)] = ye
            xn[xn_rows(i, 1), _col(t)] = yo
            if RND:
                y = [b for a in zip(_unpack(ye), _unpack(yo)) for b in a]
            a = [a * wrf[:, _col(t)] for a in y]
            r = a if r is None else [b + e for b, e in zip(r, a)]
        vpu_done(ye ^ yo)
        r = [jnp.sum(a, axis=1, keepdims=True) for a in r]
        st["xn"] = 32 * (i + 1)
        yield
        for s in range(4):
            st["r"][i // 32] = jnp.where(lane == (4 * i + s) % 128, r[s], st["r"][i // 32])
        vpu_done(lax.bitcast_convert_type(st["r"][i // 32], U32))

    def gating(i):
        half = paced(jnp.full((8, 128), 0.5, F32))
        for t in range(NT):
            e, o = [_unpack(xn[xn_rows(i, p), _col(t)]) for p in range(2)]
            for h in range(2):
                a = _pack(_silu(e[h], half), _silu(o[h], half))
                gate[t, pl.ds(16 * i + h, 8, stride=2), :] = a
        vpu_done(a)

    def product(task, k0, k1):
        half, k = pl.ds(task[1] * M // 2, M // 2), _col(k0, k1 - k0)
        wrap = gated if k0 == 0 else (lambda u: u)
        if task[0] == "qkv":
            return _nt(_bf(wrap(xn[half, k])), _bf(wt[task[2], pl.ds(task[3] * 64, 64), k]))
        return _nn(_bf(wrap(ob[half, k])), _bf(wop[pl.ds(k0 * 64, (k1 - k0) * 64), _col(task[2])]))

    def store_qkv(y, c, m, t):
        dst, off = ((qs, 0), (ks, HALO), (vs, HALO))[m]
        for p in range(2):
            dst[t, p, pl.ds(off + c * M // 2, M // 2), :] = y[p * M // 2:(p + 1) * M // 2]
            if off and c == 0:
                dst[t, p, pl.ds(0, HALO), :] = jnp.broadcast_to(y[0:1, :], (HALO, 128))

    def store_out(s, c, t):
        half, rows = pl.ds(c * M // 2, M // 2), pl.ds(c * M, M)
        g = _bf(gate[t, half, :]).astype(F32)
        y = _bf(xu[t, half, :]).astype(F32) + s * g
        if EPI:
            for a in (y[56:64], y[-8:]):
                vpu_done(lax.bitcast_convert_type(a, U32))
        outb[rows, _col(t)] = y.astype(BF)
        pltpu.make_async_copy(outb.at[rows, _col(t)], out_hbm.at[rows, _col(t)], osem).start(
            priority=1)

    def attend(jb):
        r0 = 8 * jb
        dep = st["mxu"][-1]
        for a in (st["ob"].get(jb - BACK, []) if BACK else []):
            dep = dep ^ a
        scale0 = jnp.full((8, 128), DH ** -0.5 * LOG2E, F32)
        scale = after(scale0, dep)
        win = [pl.ds(HALO + r0 - w, 8) for w in range(W)]

        def logits(par):
            q = [qs[t, par, pl.ds(r0, 8), :] * scale for t in range(NT)]
            return [_sum([q[t] * ks[t, par, r, :] for t in range(NT)]) for r in win]

        def weights(p):
            if jb == 0:
                row = lax.broadcasted_iota(I32, (8, 128), 0)
                p = [jnp.where(row >= w, a, NEG * LOG2E) for w, a in enumerate(p)]
            mx = functools.reduce(jnp.maximum, p)
            e = [jnp.exp2(a - mx) for a in p]
            return e, pltpu.reciprocal(_sum(e), full_range=False)

        def mix(par, e):
            return [_sum([a * vs[t, par, r, :] for a, r in zip(e, win)]) for t in range(NT)]

        if PK:
            ev = (lane & 32) == 0
            p = [jnp.where(ev, a, b) + pltpu.roll(jnp.where(ev, b, a), 32, 1)
                 for a, b in zip(logits(0), logits(1))]
            e, inv = weights([a + pltpu.roll(a, 64, 1) for a in p])
            e = [a * inv for a in e]
            r = [pltpu.roll(a, 32, 1) for a in e]
            o = [mix(0, [jnp.where(ev, a, b) for a, b in zip(e, r)]),
                 mix(1, [jnp.where(ev, b, a) for a, b in zip(e, r)])]
        else:
            o = []
            for par in range(2):
                p = logits(par)
                if STAG & 1:
                    scale = after(scale0, p[-1])
                p = [a + pltpu.roll(a, 64, 1) for a in p]
                e, inv = weights([a + pltpu.roll(a, 32, 1) for a in p])
                o.append([a * inv for a in mix(par, e)])
        st["ob"][jb] = [_pack(a, b) for a, b in zip(*o)]
        for t in range(NT):
            ob[pl.ds(r0, 8), _col(t)] = st["ob"][jb][t]
        vpu_done(st["ob"][jb][-1])

    def route():
        r = jnp.concatenate(_round2(*st["r"]), axis=1)
        key = jnp.where(r != r, -jnp.inf, r)
        slot = lax.broadcasted_iota(I32, (8, 256), 1)
        tok = (slot >> 2) * 32 + (slot & 3) + 4 * lax.broadcasted_iota(I32, (8, 256), 0)
        tok = tok.astype(F32)
        both = lambda f, a: f(f(a, axis=0, keepdims=True), axis=1, keepdims=True)
        full = lambda a: lax.bitcast_convert_type(jnp.broadcast_to(a, (8, 128)), U32)
        picks = []
        for _ in range(2):
            top = both(jnp.max, key)
            yield
            cand = key == top
            if picks:
                cand = cand & (tok != picks[0][0])
            idx = both(jnp.min, jnp.where(cand, tok, float(S)))
            yield
            vpu_done(full(idx))
            picks.append((idx, both(jnp.sum, jnp.where(tok == idx, r, 0.0))))
            key = jnp.where(tok == idx, -jnp.inf, key)
        picks = [(i.astype(I32), a) for i, a in picks]
        sidx = [jnp.squeeze(i) for i, _ in picks]
        base = [pl.multiple_of((i >> 4) * 8, 8) for i in sidx]
        src = [pl.multiple_of((i >> 7) * 64 + (i & 1) * 32 + ((i >> 5) & 3) * 8, 8) for i in sidx]
        yield
        row = lax.broadcasted_iota(I32, (16, 128), 0)
        xs = []
        for t in range(NT):
            sel = [jnp.sum(jnp.where(row == ((i >> 1) & 15),
                                     _bf(xn[pl.ds(b, 8), _col(t)]).astype(F32), 0.0),
                           axis=0, keepdims=True) for (i, _), b in zip(picks, src)]
            xs.append(_pack(*[jnp.broadcast_to(a, (8, 128)) for a in sel]))
        for a in xs + [full(a) for _, a in picks]:
            vpu_done(a)
        st["route"] = (picks, base, xs)

    def ffn():
        picks, base, xs = st["route"]
        span = lambda a, b: pl.ds(a * 128, min(b * 128, F) - a * 128)
        lhs = lambda us: jnp.concatenate([_bf(paced(u, -3)) for u in us], axis=1)
        hid = []
        for n0 in range(0, NF, 2):
            rem = {(i, n): _nt(lhs(xs[4:]), wf[i, span(n, n + 1), _col(4)])[:8]
                   for n in (n0, n0 + 1) for i in range(2)}
            yield
            for n in (n0, n0 + 1):
                gu = []
                for i in range(2):
                    gu.append(_nt(lhs(xs[:4]), wf[i, span(n, n + 1), _col(0, 4)])[:8] + rem[i, n])
                    yield
                g, u = _round2(*gu)
                a = _round2(_silu(g), u)[0] * u
                hid.append(_pack(a, a))
        y = y4 = None
        for n in range(NF):
            a = _nn(lhs(hid[n:n + 1]), wf[2, span(n, n + 1), _col(0, 4)])[:8]
            y = a if y is None else y + a
            yield
        for n0 in range(0, NF, 4):
            a = _nn(lhs(hid[n0:n0 + 4]), wf[2, span(n0, min(n0 + 4, NF)), _col(4)])[:8]
            y4 = a if y4 is None else y4 + a
            yield
        y = _round(jnp.concatenate([y, y4], axis=1))
        assert st["gated"] == S // 32
        row = lax.broadcasted_iota(I32, (8, 128), 0)
        for j, (idx, val) in enumerate(picks):
            upd = _round(y[2 * j:2 * j + 1] * _round(jax.nn.sigmoid(val)))
            for t in range(NT):
                g = _silu(_round(_unpack(xs[t])[j] + upd[:, t * 128:(t + 1) * 128]))
                cur = _unpack(gate[t, pl.ds(base[j], 8), :])
                gate[t, pl.ds(base[j], 8), :] = _pack(
                    *[jnp.where(2 * row + p == (idx & 15), g, a) for p, a in enumerate(cur)])

    for cp in (wrcopy, xcopy[0], kcopy[0], kcopy[1], xcopy[1], xcopy[2], vcopy):
        cp.start()
    wait(xcopy[0])
    wait(wrcopy)
    wrf[...] = jnp.broadcast_to(wrb[...].astype(F32).reshape(1, D), (8, D))
    st["never"] = (lax.bitcast_convert_type(wrf[:, _col(0)], I32) & 0xFFFF) != 0
    started = XCUT[1] // 32
    live = [norm(i) for i in range(started)]
    while live:
        live = [g for g in live if not _advance(g)]
    for cp, a, b in zip(kcopy, KCUT[:-1], KCUT[1:]):
        wait(cp)
        for f in (prep_a, prep_b):
            for t in range(a // 128, b // 128):
                f(1, t)
    wait(xcopy[1])
    live = [norm(started + i) for i in range(M // 32)]
    started += M // 32
    live = [g for g in live if not _advance(g)]

    order = _slot_order()
    app = M // 16
    need = {t[1]: s - s % 4 for s, t in enumerate(order) if t[0] == "proj" and t[2] == 0}
    avail = {t[1]: s for s, t in enumerate(order) if t[0] == "qkv" and t[2:] == (0, NT - 1)}
    waits = {B1: [xcopy[2]], B2: [vcopy], B3: [xcopy[3], qcopy], FFN_AT: [fcopy]}
    starts = {B1: [xcopy[3], qcopy], F0: [fcopy]}
    arrived = {B1: (XCUT[3], LN1_DUE), B3: (XCUT[4], LN2_DUE)}
    extra = {}
    for t in range(NT):
        for s, f, args in ((B2 + t, prep_a, (2, t)), (B2 + 1 + t, prep_b, (2, t)),
                           (B3 + t, prep_a, (0, t)), (B3 + 2 + t, prep_b, (0, t)),
                           (FFN_AT + 5 * t, prep_wo, (t,))):
            extra.setdefault(s, []).append(functools.partial(f, *args))

    routeg, ffng = route(), ffn()
    route_done = ffn_done = False
    xrows, xdue = XCUT[2], LN0_DUE
    attended = 0
    lcredit = gcredit = acredit = 0.0
    for slot, task in enumerate(order):
        if slot % 4 == 0:
            for u in order[slot:slot + 4]:
                assert (st["xn"] >= (u[1] + 1) * M if u[0] == "qkv"
                        else attended >= (u[1] + 1) * app), (slot, u)
            rem = [product(u, 4, NT) for u in order[slot:slot + 4]]
        y = product(task, 0, 4) + rem[slot % 4]
        mxu_done(y[-8:])
        if task[0] == "qkv":
            store_qkv(y, *task[1:])
        else:
            assert ffn_done
            store_out(y, *task[1:])
        for cp in waits.get(slot, []):
            wait(cp)
        for cp in starts.get(slot, []):
            cp.start()
        xrows, xdue = arrived.get(slot, (xrows, xdue))

        if slot >= FFN_AT and not ffn_done:
            assert route_done
            ffn_done = _advance(ffng)
        if started == S // 32 and not live and not route_done and slot % RS == 0:
            route_done = _advance(routeg)
        lcredit = min(lcredit + (xrows // 32 - started) / max(xdue - slot, 1), 1.0)
        if lcredit >= 0.999 and started < xrows // 32:
            lcredit -= 1
            live.append(norm(started))
            started += 1
        live = [g for g in live if not _advance(g)]

        for lim, s0, s1 in ((XCUT[3] // 32, NT * NK, B3),
                            (S // 32, G0, FFN_AT + FFN_LEN - 10)):
            if s0 <= slot and st["gated"] < lim:
                gcredit += (lim - st["gated"]) / max(s1 - slot, 1)
                while gcredit >= 0.999 and st["gated"] < lim:
                    gcredit -= 1
                    gating(st["gated"])
                    st["gated"] += 1
                break

        ready = sum(app for c in avail if avail[c] + LAG <= slot)
        rate = max((c + 1) * app - attended for c in need) and max(
            ((c + 1) * app - attended) / max(need[c] - 3 - LAG - slot, 1) for c in need)
        acredit += rate if slot > LN2_DUE else min(rate, A1)
        while acredit >= PAIR and attended < ready:
            acredit -= PAIR
            for _ in range(PAIR):
                attend(attended)
                attended += 1
        acredit = min(acredit, PAIR)
        for f in extra.get(slot, []):
            f()
    pltpu.make_async_copy(outb, out_hbm, osem).wait()


@jax.jit
def pallas_recurrent_scan__sliding_local_dilated__moe_arch_mod__prompt_kernel(
    A_x, A_wqkv, A_wo, B_x, B_w_r, B_w_gate, B_w_up, B_w_down,
):
    del B_x
    hbm = pl.BlockSpec(memory_space=pltpu.HBM)
    V = pltpu.VMEM
    out = pl.pallas_call(
        _kernel,
        in_specs=[hbm] * 7,
        out_specs=hbm,
        out_shape=jax.ShapeDtypeStruct((S, D), BF),
        scratch_shapes=[
            V((NT, S, 128), BF),
            V((4, D, D), BF),
            V((D,), BF),
            V((8, D), F32),
            V((3, F, D), BF),
            V((4 * NT, D // 2, 128), U32),
            V((3, D // 2, D), U32),
            V((D // 2, D), U32),
            V((S // 2, D), U32),
            V((NT, S // 2, 128), U32),
            V((NT, 2, S // 2, 128), F32),
            V((NT, 2, HALO + S // 2, 128), F32),
            V((NT, 2, HALO + S // 2, 128), F32),
            V((S // 2, D), U32),
            V((S, D), BF),
            pltpu.SemaphoreType.DMA((5 + len(XCUT),)),
            pltpu.SemaphoreType.DMA(()),
        ],
        compiler_params=pltpu.CompilerParams(vmem_limit_bytes=100 << 20),
        name="fused",
    )(A_x.reshape(S, D), A_wqkv, A_wo, B_w_r, B_w_gate.T, B_w_up.T, B_w_down)
    return out.reshape(1, S, D)
```

```python
import functools

import jax
import jax.numpy as jnp
import numpy as np
from jax import lax
from jax.experimental import pallas as pl
from jax.experimental.pallas import tpu as pltpu


S, D, F = 2048, 640, 1728
H, DH, W = 32, 20, 8
NT = D // 128
NF = -(-F // 128)
HALO = 8
BF, F32, U32, I32 = jnp.bfloat16, jnp.float32, jnp.uint32, jnp.int32
LOG2E = 1.4426950408889634
NEG = -998244352.0
EPS = 1.0013580322265625e-05

M = 128
NC = S // M
NK = 6
XCUT = (0, 128, 384, NK * M, S)
KCUT = (0, 384, D)
B1 = 6
B2 = 21
B3 = 50
F0 = 40
FFN_AT = 180
FFN_LEN = 60
LN0_DUE = 4
LN1_DUE = 18
LN2_DUE = 156
TAIL = 3
LAG = 2
REV = 7
BACK = 3
PAIR = 1
A1 = 0.43
PK = 0
RND = 1
P0 = 1
DELAY = 0
RS = 3
G0 = 170
G32 = 0
SCOPE = 0


def _pack(a, b):
    return pltpu.pack_elementwise([a, b], packed_dtype=BF)


def _unpack(u):
    return [pltpu.unpack_elementwise(u, index=i, packed_dtype=BF, unpacked_dtype=F32)
            for i in range(2)]


def _round2(a, b):
    return _unpack(_pack(a, b))


def _round4(v):
    return _round2(v[0], v[1]) + _round2(v[2], v[3])


def _round(x):
    return x.astype(BF).astype(F32)


def _nt(a, b):
    return lax.dot_general(a, b, (((1,), (1,)), ((), ())), preferred_element_type=F32)


def _nn(a, b):
    return lax.dot_general(a, b, (((1,), (0,)), ((), ())), preferred_element_type=F32)


def _bf(u):
    return pltpu.bitcast(u, BF)


def _silu(x, half=0.5):
    h = x * half
    return h * jnp.tanh(h) + h


def _sum(xs):
    return functools.reduce(jnp.add, xs)


def _col(t, n=1):
    return pl.ds(t * 128, n * 128)


def _advance(g):
    return next(g, "end") == "end"


class _Copies:
    def __init__(self, pairs, sem, pri=P0):
        self.pri = pri
        self.cs = [pltpu.make_async_copy(a, b, sem) for a, b in pairs]

    def start(self):
        for c in self.cs:
            c.start(priority=self.pri)

    def wait(self):
        for c in self.cs:
            c.wait()


def _slot_order():
    tiles = lambda c, m: [("qkv", c, m, t) for t in range(NT)]
    order = [a for m in (1, 2, 0) for c in range(NK) for a in tiles(c, m)]
    order += [a for c in range(NK, NC) for m in (1, 2, 0) for a in tiles(c, m)]
    order, a = order[:FFN_AT + FFN_LEN], order[FFN_AT + FFN_LEN:]
    projs = [("proj", c, t) for c in range(NC) for t in range(NT)]
    b = projs[:-TAIL * NT]
    i = j = 0
    while i < len(a) or j < len(b):
        if j >= len(b) or (i < len(a) and i * len(b) < j * len(a)):
            order += a[i:i + NT]
            i += NT
        else:
            order += b[j:j + NT]
            j += NT
    return order + projs[-TAIL * NT:]


def _kernel(x_hbm, wqkv_hbm, wo_hbm, wr_hbm, wg_hbm, wu_hbm, wd_hbm, out_hbm,
            xb, wraw, wrb, wrf, wf, stage, wt, wop, xn, gate, qs, ks, vs, ob, outb,
            wsem, osem):
    xu = xb.bitcast(U32)
    xcopy = [_Copies([(x_hbm.at[pl.ds(a, b - a), _col(t)], xb.at[t, pl.ds(a, b - a)])
                      for t in range(NT)], wsem.at[6 + i])
             for i, (a, b) in enumerate(zip(XCUT[:-1], XCUT[1:]))]

    def wcopy(m, a, b, sem):
        return _Copies([(wqkv_hbm.at[pl.ds(a, b - a), _col(m * NT, NT)],
                         wraw.at[m, pl.ds(a, b - a)])], wsem.at[sem])

    kcopy = [wcopy(1, KCUT[0], KCUT[1], 0), wcopy(1, KCUT[1], KCUT[2], 1)]
    vcopy = wcopy(2, 0, D, 2)
    qcopy = wcopy(0, 0, D, 3)
    wrcopy = _Copies([(wr_hbm, wrb)], wsem.at[4])
    fcopy = _Copies([(wo_hbm, wraw.at[3])] + [
        (w.at[:, _col(t)], wf.at[i * NT + t])
        for i, w in enumerate((wg_hbm, wu_hbm, wd_hbm)) for t in range(NT)], wsem.at[5], 1)
    wfu = wf.bitcast(U32)

    lane = lax.broadcasted_iota(I32, (8, 128), 1)
    st = {"r": [jnp.zeros((8, 128), F32)] * 2, "xn": 0, "gated": 0,
          "mxu": [], "vpu": None, "hist": [], "ob": {}}

    def wait(cp):
        if SCOPE:
            st["nw"] = st.get("nw", 0) + 1
            with jax.named_scope(f"w{st['nw']:02d}"):
                cp.wait()
        else:
            cp.wait()

    def after(v, dep):
        n = v.shape[1]
        return jnp.where(st["never"][:, :n], lax.bitcast_convert_type(dep, v.dtype)[:, :n], v)

    def mxu_done(v):
        v = lax.bitcast_convert_type(v, U32)
        st["mxu"].append(v ^ st["mxu"][-1] if st["mxu"] else v)

    def vpu_done(v):
        st["vpu"] = v if st["vpu"] is None else v ^ st["vpu"]

    def paced(v, age=-1):
        return after(v, st["mxu"][age]) if st["mxu"] else v

    def gated(u):
        st["hist"].append(st["vpu"])
        if len(st["hist"]) <= REV:
            return u
        head = jnp.concatenate([after(u[:8, :128], st["hist"][-1 - REV]), u[:8, 128:]], axis=1)
        return jnp.concatenate([head, u[8:]], axis=0)

    def permute_rows(src, dst, t):
        for d2 in range(DH // 2):
            u = src[pl.ds(d2, H // 2, stride=DH), :]
            v = src[pl.ds(d2 + DH // 2, H // 2, stride=DH), :]
            dst[pl.ds(H * d2, H // 2), _col(t)] = pltpu.pack_elementwise([u, v], packed_dtype=jnp.uint16)
            dst[pl.ds(H * d2 + H // 2, H // 2), _col(t)] = pltpu.pack_elementwise(
                [u >> 16, v >> 16], packed_dtype=jnp.uint16)

    def prep_a(m, t):
        stage[m * NT + t] = pltpu.bitcast(wraw[m, _col(t), :].T, U32)

    def prep_b(m, t):
        permute_rows(stage.at[m * NT + t], wt.at[m], t)

    def prep_wo(t):
        stage[3 * NT + t] = pltpu.bitcast(wraw[3, :, _col(t)], U32)
        permute_rows(stage.at[3 * NT + t], wop, t)

    def xn_rows(i, par):
        c, j = divmod(i, M // 32)
        return pl.ds(c * M // 2 + par * M // 4 + 8 * j, 8)

    def norm(i):
        def load(t):
            return (_unpack(xu[t, pl.ds(16 * i, 8, stride=2), :])
                    + _unpack(xu[t, pl.ds(16 * i + 1, 8, stride=2), :]))

        x = [load(t) for t in range(NT)]
        x[0] = [paced(a) for a in x[0]]
        tot, ml, m2 = [], [], []
        for xs in zip(*x):
            s = _sum(xs)
            tot.append(jnp.sum(s, axis=1, keepdims=True))
            ml.append(s * (1.0 / NT))
            m2.append(_sum([(a - ml[-1]) * (a - ml[-1]) for a in xs]))
        yield
        mean = [jnp.broadcast_to(a, (8, 128)) * (1.0 / D) for a in tot]
        tot = [jnp.sum(b + ((a - m) * (a - m)) * float(NT), axis=1, keepdims=True)
               for a, b, m in zip(ml, m2, mean)]
        mean = [_pack(mean[0], mean[1]), _pack(mean[2], mean[3])]
        yield
        var = _round4([jnp.broadcast_to(a, (8, 128)) * (1.0 / D) for a in tot])
        var = _round4([a + EPS for a in var])
        sd = _round4([a * lax.rsqrt(a) for a in var])
        inv = [jnp.where(a == jnp.inf, 0.0, pltpu.reciprocal(b, full_range=False))
               for a, b in zip(var, sd)]
        mean = _unpack(mean[0]) + _unpack(mean[1])
        r = None
        for t in range(NT):
            y = [a - m for a, m in zip(load(t), mean)]
            y = [a * b for a, b in zip(_round4(y) if RND else y, inv)]
            ye, yo = _pack(y[0], y[2]), _pack(y[1], y[3])
            xn[xn_rows(i, 0), _col(t)] = ye
            xn[xn_rows(i, 1), _col(t)] = yo
            if RND:
                y = [b for a in zip(_unpack(ye), _unpack(yo)) for b in a]
            a = [a * wrf[:, _col(t)] for a in y]
            r = a if r is None else [b + e for b, e in zip(r, a)]
        vpu_done(ye ^ yo)
        r = [jnp.sum(a, axis=1, keepdims=True) for a in r]
        st["xn"] = 32 * (i + 1)
        yield
        for s in range(4):
            st["r"][i // 32] = jnp.where(lane == (4 * i + s) % 128, r[s], st["r"][i // 32])
        vpu_done(lax.bitcast_convert_type(st["r"][i // 32], U32))

    def gating(i):
        half = paced(jnp.full((8, 128), 0.5, F32))
        for t in range(NT):
            if G32:
                for p in range(2):
                    a = _silu(_bf(xn[xn_rows(i, p), _col(t)]).astype(F32),
                              jnp.concatenate([half, half], axis=0))
                    gate[t, pl.ds(32 * i + p, 16, stride=2), :] = a
                a = lax.bitcast_convert_type(a[8:], U32)
                continue
            e, o = [_unpack(xn[xn_rows(i, p), _col(t)]) for p in range(2)]
            for h in range(2):
                a = _pack(_silu(e[h], half), _silu(o[h], half))
                gate[t, pl.ds(16 * i + h, 8, stride=2), :] = a
        vpu_done(a)

    def product(task, k0, k1):
        half, k = pl.ds(task[1] * M // 2, M // 2), _col(k0, k1 - k0)
        wrap = gated if k0 == 0 else (lambda u: u)
        if task[0] == "qkv":
            return _nt(_bf(wrap(xn[half, k])), _bf(wt[task[2], pl.ds(task[3] * 64, 64), k]))
        return _nn(_bf(wrap(ob[half, k])), _bf(wop[pl.ds(k0 * 64, (k1 - k0) * 64), _col(task[2])]))

    def store_qkv(y, c, m, t):
        dst, off = ((qs, 0), (ks, HALO), (vs, HALO))[m]
        for p in range(2):
            dst[t, p, pl.ds(off + c * M // 2, M // 2), :] = y[p * M // 2:(p + 1) * M // 2]
            if off and c == 0:
                dst[t, p, pl.ds(0, HALO), :] = jnp.broadcast_to(y[0:1, :], (HALO, 128))

    def store_out(s, c, t):
        half, rows = pl.ds(c * M // 2, M // 2), pl.ds(c * M, M)
        g = gate[t, rows, :] if G32 else _bf(gate[t, half, :]).astype(F32)
        y = _bf(xu[t, half, :]).astype(F32) + s * g
        outb[rows, _col(t)] = y.astype(BF)
        pltpu.make_async_copy(outb.at[rows, _col(t)], out_hbm.at[rows, _col(t)], osem).start(
            priority=1)

    def attend(jb):
        r0 = 8 * jb
        dep = st["mxu"][-1]
        for a in (st["ob"].get(jb - BACK, []) if BACK else []):
            dep = dep ^ a
        scale = after(jnp.full((8, 128), DH ** -0.5 * LOG2E, F32), dep)
        win = [pl.ds(HALO + r0 - w, 8) for w in range(W)]

        def logits(par):
            q = [qs[t, par, pl.ds(r0, 8), :] * scale for t in range(NT)]
            return [_sum([q[t] * ks[t, par, r, :] for t in range(NT)]) for r in win]

        def weights(p):
            if jb == 0:
                row = lax.broadcasted_iota(I32, (8, 128), 0)
                p = [jnp.where(row >= w, a, NEG * LOG2E) for w, a in enumerate(p)]
            mx = functools.reduce(jnp.maximum, p)
            e = [jnp.exp2(a - mx) for a in p]
            return e, pltpu.reciprocal(_sum(e), full_range=False)

        def mix(par, e):
            return [_sum([a * vs[t, par, r, :] for a, r in zip(e, win)]) for t in range(NT)]

        if PK:
            ev = (lane & 32) == 0
            p = [jnp.where(ev, a, b) + pltpu.roll(jnp.where(ev, b, a), 32, 1)
                 for a, b in zip(logits(0), logits(1))]
            e, inv = weights([a + pltpu.roll(a, 64, 1) for a in p])
            e = [a * inv for a in e]
            r = [pltpu.roll(a, 32, 1) for a in e]
            o = [mix(0, [jnp.where(ev, a, b) for a, b in zip(e, r)]),
                 mix(1, [jnp.where(ev, b, a) for a, b in zip(e, r)])]
        else:
            o = []
            for par in range(2):
                p = [a + pltpu.roll(a, 64, 1) for a in logits(par)]
                e, inv = weights([a + pltpu.roll(a, 32, 1) for a in p])
                o.append([a * inv for a in mix(par, e)])
        st["ob"][jb] = [_pack(a, b) for a, b in zip(*o)]
        for t in range(NT):
            ob[pl.ds(r0, 8), _col(t)] = st["ob"][jb][t]
        vpu_done(st["ob"][jb][-1])

    def route():
        r = jnp.concatenate(_round2(*st["r"]), axis=1)
        key = jnp.where(r != r, -jnp.inf, r)
        slot = lax.broadcasted_iota(I32, (8, 256), 1)
        tok = (slot >> 2) * 32 + (slot & 3) + 4 * lax.broadcasted_iota(I32, (8, 256), 0)
        tok = tok.astype(F32)
        both = lambda f, a: f(f(a, axis=0, keepdims=True), axis=1, keepdims=True)
        full = lambda a: lax.bitcast_convert_type(jnp.broadcast_to(a, (8, 128)), U32)
        picks = []
        for _ in range(2):
            top = both(jnp.max, key)
            yield
            cand = key == top
            if picks:
                cand = cand & (tok != picks[0][0])
            idx = both(jnp.min, jnp.where(cand, tok, float(S)))
            yield
            vpu_done(full(idx))
            picks.append((idx, both(jnp.sum, jnp.where(tok == idx, r, 0.0))))
            key = jnp.where(tok == idx, -jnp.inf, key)
        picks = [(i.astype(I32), a) for i, a in picks]
        sidx = [jnp.squeeze(i) for i, _ in picks]
        base = [pl.multiple_of((i >> (3 if G32 else 4)) * 8, 8) for i in sidx]
        src = [pl.multiple_of((i >> 7) * 64 + (i & 1) * 32 + ((i >> 5) & 3) * 8, 8) for i in sidx]
        yield
        row = lax.broadcasted_iota(I32, (16, 128), 0)
        odd = (lax.broadcasted_iota(I32, (8, 128), 0) & 1) == 1
        xs = []
        for t in range(NT):
            sel = [jnp.sum(jnp.where(row == ((i >> 1) & 15),
                                     _bf(xn[pl.ds(b, 8), _col(t)]).astype(F32), 0.0),
                           axis=0, keepdims=True) for (i, _), b in zip(picks, src)]
            xs.append(jnp.where(odd, sel[1], sel[0]))
        for a in xs + [a for _, a in picks]:
            vpu_done(full(a))
        st["route"] = (picks, base, xs)

    def ffn():
        picks, base, xs = st["route"]
        lhs = lambda us: jnp.concatenate([paced(u, -3) for u in us], axis=1)

        def rhs(i, n0, n1, ts):
            rows = pl.ds(n0 * 64, min(n1 * 64, F // 2) - n0 * 64)
            return jnp.concatenate([_bf(wfu[i * NT + t, rows, :]) for t in ts], axis=1)

        hid = []
        for n0 in range(0, NF, 2):
            rem = {(i, n): _nt(lhs(xs[4:]), rhs(i, n, n + 1, [4]))
                   for n in (n0, n0 + 1) for i in range(2)}
            yield
            for n in (n0, n0 + 1):
                gu = []
                for i in range(2):
                    gu.append(_nt(lhs(xs[:4]), rhs(i, n, n + 1, range(4))) + rem[i, n])
                    yield
                g, u = _round2(*gu)
                hid.append(_round(_round(_silu(g)) * u))
        y = y4 = None
        for n in range(NF):
            a = _nn(lhs(hid[n:n + 1]), rhs(2, n, n + 1, range(4)))
            y = a if y is None else y + a
            yield
        for n0 in range(0, NF, 4):
            a = _nn(lhs(hid[n0:n0 + 4]), rhs(2, n0, n0 + 4, [4]))
            y4 = a if y4 is None else y4 + a
            yield
        y = _round(jnp.concatenate([y, y4], axis=1))
        assert st["gated"] == S // 32
        row = lax.broadcasted_iota(I32, (8, 128), 0)
        for j, (idx, val) in enumerate(picks):
            upd = _round(y[j:j + 1] * _round(jax.nn.sigmoid(val)))
            for t in range(NT):
                g = _silu(_round(xs[t][j:j + 1] + upd[:, t * 128:(t + 1) * 128]))
                if G32:
                    b = pl.ds(base[j], 8)
                    gate[t, b, :] = jnp.where(row == (idx & 7), g, gate[t, b, :])
                    continue
                cur = _unpack(gate[t, pl.ds(base[j], 8), :])
                gate[t, pl.ds(base[j], 8), :] = _pack(
                    *[jnp.where(2 * row + p == (idx & 15), g, a) for p, a in enumerate(cur)])

    for cp in (wrcopy, xcopy[0], kcopy[0], kcopy[1], xcopy[1], xcopy[2], vcopy):
        cp.start()
    wait(xcopy[0])
    wait(wrcopy)
    wrf[...] = jnp.broadcast_to(wrb[...].astype(F32).reshape(1, D), (8, D))
    st["never"] = (lax.bitcast_convert_type(wrf[:, _col(0)], I32) & 0xFFFF) != 0
    started = XCUT[1] // 32
    live = [norm(i) for i in range(started)]
    while live:
        live = [g for g in live if not _advance(g)]
    for cp, a, b in zip(kcopy, KCUT[:-1], KCUT[1:]):
        wait(cp)
        for f in (prep_a, prep_b):
            for t in range(a // 128, b // 128):
                f(1, t)
    wait(xcopy[1])
    live = [norm(started + i) for i in range(M // 32)]
    started += M // 32
    live = [g for g in live if not _advance(g)]

    order = _slot_order()
    app = M // 16
    need = {t[1]: s - s % 4 for s, t in enumerate(order) if t[0] == "proj" and t[2] == 0}
    avail = {t[1]: s for s, t in enumerate(order) if t[0] == "qkv" and t[2:] == (0, NT - 1)}
    waits = {B1: [xcopy[2]], B2: [vcopy], B3: [xcopy[3], qcopy], FFN_AT: [fcopy]}
    starts = {B1: [xcopy[3], qcopy], F0: [fcopy]}
    arrived = {B1: (XCUT[3], LN1_DUE), B3: (XCUT[4], LN2_DUE)}
    extra = {}
    for t in range(NT):
        for s, f, args in ((B2 + t, prep_a, (2, t)), (B2 + 1 + t, prep_b, (2, t)),
                           (B3 + t, prep_a, (0, t)), (B3 + 2 + t, prep_b, (0, t)),
                           (FFN_AT + 5 * t, prep_wo, (t,))):
            extra.setdefault(s, []).append(functools.partial(f, *args))

    routeg, ffng = route(), ffn()
    route_done = ffn_done = False
    xrows, xdue = XCUT[2], LN0_DUE
    attended = 0
    lcredit = gcredit = acredit = 0.0
    for slot, task in enumerate(order):
        if slot % 4 == 0:
            for u in order[slot:slot + 4]:
                assert (st["xn"] >= (u[1] + 1) * M if u[0] == "qkv"
                        else attended >= (u[1] + 1) * app), (slot, u)
            rem = [product(u, 4, NT) for u in order[slot:slot + 4]]
        y = product(task, 0, 4) + rem[slot % 4]
        mxu_done(y[-8:])
        if task[0] == "qkv":
            store_qkv(y, *task[1:])
        else:
            assert ffn_done
            store_out(y, *task[1:])
        for cp in waits.get(slot, []):
            wait(cp)
        for cp in starts.get(slot, []):
            cp.start()
        xrows, xdue = arrived.get(slot, (xrows, xdue))

        if slot >= FFN_AT and not ffn_done:
            assert route_done
            ffn_done = _advance(ffng)
        if started == S // 32 and not live and not route_done and slot % RS == 0:
            route_done = _advance(routeg)
        lcredit = min(lcredit + (xrows // 32 - started) / max(xdue - slot, 1), 1.0)
        if lcredit >= 0.999 and started < xrows // 32:
            lcredit -= 1
            live.append(norm(started))
            started += 1
        live = [g for g in live if not _advance(g)]

        for lim, s0, s1 in ((XCUT[3] // 32, NT * NK, B3),
                            (S // 32, G0, FFN_AT + FFN_LEN - 10)):
            if s0 <= slot and st["gated"] < lim:
                gcredit += (lim - st["gated"]) / max(s1 - slot, 1)
                while gcredit >= 0.999 and st["gated"] < lim:
                    gcredit -= 1
                    gating(st["gated"])
                    st["gated"] += 1
                break

        ready = sum(app for c in avail if avail[c] + LAG <= slot)
        rate = max((c + 1) * app - attended for c in need) and max(
            ((c + 1) * app - attended) / max(need[c] - 3 - LAG - slot, 1) for c in need)
        acredit += rate if slot > LN2_DUE else min(rate, A1)
        while acredit >= PAIR and attended < ready:
            acredit -= PAIR
            for _ in range(PAIR):
                attend(attended)
                attended += 1
        acredit = min(acredit, PAIR)
        for f in extra.get(slot, []):
            f()
    pltpu.make_async_copy(outb, out_hbm, osem).wait()


@jax.jit
def pallas_recurrent_scan__sliding_local_dilated__moe_arch_mod__prompt_kernel(
    A_x, A_wqkv, A_wo, B_x, B_w_r, B_w_gate, B_w_up, B_w_down,
):
    del B_x
    hbm = pl.BlockSpec(memory_space=pltpu.HBM)
    V = pltpu.VMEM
    out = pl.pallas_call(
        _kernel,
        in_specs=[hbm] * 7,
        out_specs=hbm,
        out_shape=jax.ShapeDtypeStruct((S, D), BF),
        scratch_shapes=[
            V((NT, S, 128), BF),
            V((4, D, D), BF),
            V((D,), BF),
            V((8, D), F32),
            V((3 * NT, F, 128), BF),
            V((4 * NT, D // 2, 128), U32),
            V((3, D // 2, D), U32),
            V((D // 2, D), U32),
            V((S // 2, D), U32),
            V((NT, S, 128), F32) if G32 else V((NT, S // 2, 128), U32),
            V((NT, 2, S // 2, 128), F32),
            V((NT, 2, HALO + S // 2, 128), F32),
            V((NT, 2, HALO + S // 2, 128), F32),
            V((S // 2, D), U32),
            V((S, D), BF),
            pltpu.SemaphoreType.DMA((5 + len(XCUT),)),
            pltpu.SemaphoreType.DMA(()),
        ],
        compiler_params=pltpu.CompilerParams(vmem_limit_bytes=100 << 20),
        name="fused",
    )(A_x.reshape(S, D), A_wqkv, A_wo, B_w_r, B_w_gate.T, B_w_up.T, B_w_down)
    return out.reshape(1, S, D)
```

```python
import functools

import jax
import jax.numpy as jnp
import numpy as np
from jax import lax
from jax.experimental import pallas as pl
from jax.experimental.pallas import tpu as pltpu


S, D, F = 2048, 640, 1728
H, DH, W, DIL = 32, 20, 8, 2
NT = D // 128
NF = -(-F // 128)
HALO = 16
BF, F32, U32, I32 = jnp.bfloat16, jnp.float32, jnp.uint32, jnp.int32
LOG2E = 1.4426950408889634
NEG = -998244352.0
EPS = 1.0013580322265625e-05

M = 128
NC = S // M
NK = 6
XCUT = (0, 128, 384, NK * M, S)
KCUT = (0, 384, D)
B1 = 6
B2 = 18
B3 = 50
F0 = 40
FFN_AT = 180
FFN_LEN = 60
LN0_DUE = 4
LN1_DUE = 18
LN2_DUE = 156
TAIL = 3
LAG = 2
REV = 12
BACK = 3
PAIR = 1
A1 = 0.43
RS = 3
G0 = 120
G1 = 234
NO = 2


def _round2(a, b):
    c = _round(jnp.concatenate([a, b], axis=1))
    return [c[:, :a.shape[1]], c[:, a.shape[1]:]]


def _round4(v):
    return _round2(v[0], v[1]) + _round2(v[2], v[3])


def _round(x):
    return x.astype(BF).astype(F32)


def _nt(a, b):
    return lax.dot_general(a, b, (((1,), (1,)), ((), ())), preferred_element_type=F32)


def _nn(a, b):
    return lax.dot_general(a, b, (((1,), (0,)), ((), ())), preferred_element_type=F32)


def _bf(u):
    return pltpu.bitcast(u, BF)


def _silu(x, half=0.5):
    h = x * half
    return h * jnp.tanh(h) + h


def _sum(xs):
    return functools.reduce(jnp.add, xs)


def _col(t, n=1):
    return pl.ds(t * 128, n * 128)


def _advance(g):
    return next(g, "end") == "end"


class _Copies:
    def __init__(self, pairs, sem):
        self.cs = [pltpu.make_async_copy(a, b, sem) for a, b in pairs]

    def start(self):
        for c in self.cs:
            c.start(priority=1)

    def wait(self):
        for c in self.cs:
            c.wait()


def _slot_order():
    tiles = lambda c, m: [("qkv", c, m, t) for t in range(NT)]
    order = [a for m in (1, 2, 0) for c in range(NK) for a in tiles(c, m)]
    order += [a for c in range(NK, NC) for m in (1, 2, 0) for a in tiles(c, m)]
    order, a = order[:FFN_AT + FFN_LEN], order[FFN_AT + FFN_LEN:]
    projs = [("proj", c, t) for c in range(NC) for t in range(NT)]
    b = projs[:-TAIL * NT]
    i = j = 0
    while i < len(a) or j < len(b):
        if j >= len(b) or (i < len(a) and i * len(b) < j * len(a)):
            order += a[i:i + NT]
            i += NT
        else:
            order += b[j:j + NT]
            j += NT
    return order + projs[-TAIL * NT:]


def _kernel(x_hbm, wqkv_hbm, wo_hbm, wr_hbm, wg_hbm, wu_hbm, wd_hbm, out_hbm,
            xb, kraw, vraw, qraw, oraw, wrb, wrf, wf, stage, wt, wop, xn, gate, qs, ks, vs, ob, outb,
            wsem, osem):
    xu = [b.bitcast(U32) for b in xb]
    xnu, obu = xn.bitcast(U32), ob.bitcast(U32)
    xcopy = [_Copies([(x_hbm.at[pl.ds(a, b - a), _col(t)], xb[i].at[t]) for t in range(NT)],
                     wsem.at[6 + i])
             for i, (a, b) in enumerate(zip(XCUT[:-1], XCUT[1:]))]

    def x_rows(t, r0, n):
        i = max(j for j, a in enumerate(XCUT) if a <= r0)
        return _bf(xu[i][t, pl.ds((r0 - XCUT[i]) // 2, n // 2), :]).astype(F32)

    kcopy = [_Copies([(wqkv_hbm.at[pl.ds(a, b - a), _col(NT, NT)], kraw[i])], wsem.at[i])
             for i, (a, b) in enumerate(zip(KCUT[:-1], KCUT[1:]))]
    vcopy = _Copies([(wqkv_hbm.at[:, _col(2 * NT, NT)], vraw)], wsem.at[2])
    qcopy = _Copies([(wqkv_hbm.at[:, _col(0, NT)], qraw)], wsem.at[3])
    wrcopy = _Copies([(wr_hbm, wrb)], wsem.at[4])
    fcopy = _Copies([(wo_hbm, oraw)] + [
        (w.at[:, _col(t)], wf.at[i * NT + t])
        for i, w in enumerate((wg_hbm, wu_hbm, wd_hbm)) for t in range(NT)], wsem.at[5])
    wfu = wf.bitcast(U32)

    lane = lax.broadcasted_iota(I32, (8, 128), 1)
    st = {"r": [jnp.zeros((8, 128), F32)] * 2, "xn": 0, "gated": 0,
          "mxu": [], "vpu": None, "hist": [], "out": {}}

    def after(v, dep):
        n = v.shape[1]
        return jnp.where(st["never"][:, :n], lax.bitcast_convert_type(dep, v.dtype)[:, :n], v)

    def mxu_done(v):
        v = lax.bitcast_convert_type(v, U32)
        st["mxu"].append(v ^ st["mxu"][-1] if st["mxu"] else v)

    def vpu_done(v):
        st["vpu"] = v if st["vpu"] is None else v ^ st["vpu"]

    def paced(v, age=-1):
        return after(v, st["mxu"][age]) if st["mxu"] else v

    def gated(u):
        st["hist"].append(st["vpu"])
        if len(st["hist"]) <= REV:
            return u
        head = jnp.concatenate([after(u[:8, :128], st["hist"][-1 - REV]), u[:8, 128:]], axis=1)
        return jnp.concatenate([head, u[8:]], axis=0)

    def permute_rows(src, dst, t):
        for d2 in range(DH // 2):
            u = src[pl.ds(d2, H // 2, stride=DH), :]
            v = src[pl.ds(d2 + DH // 2, H // 2, stride=DH), :]
            dst[pl.ds(H * d2, H // 2), _col(t)] = (u & np.uint32(0xFFFF)) | (v << 16)
            dst[pl.ds(H * d2 + H // 2, H // 2), _col(t)] = (u >> 16) | (v & np.uint32(0xFFFF0000))

    def prep_a(m, t):
        src, r0 = (qraw, 0) if m == 0 else (vraw, 0)
        if m == 1:
            i = int(t * 128 >= KCUT[1])
            src, r0 = kraw[i], KCUT[i]
        stage[m * NT + t, pl.ds(0, D // 2), :] = pltpu.bitcast(
            src[pl.ds(t * 128 - r0, 128), :].T, U32)

    def prep_b(m, t):
        permute_rows(stage.at[m * NT + t], wt.at[m], t)

    def prep_wo(t):
        stage[3 * NT + t, pl.ds(0, D // 2), :] = pltpu.bitcast(oraw[:, _col(t)], U32)
        permute_rows(stage.at[3 * NT + t], wop, t)

    def norm(i):
        def load(t):
            a = x_rows(t, 32 * i, 32)
            return [a[8 * s:8 * s + 8] for s in range(4)]

        x = [load(t) for t in range(NT)]
        x[0] = [paced(a) for a in x[0]]
        tot, ml, m2 = [], [], []
        for xs in zip(*x):
            s = _sum(xs)
            tot.append(jnp.sum(s, axis=1, keepdims=True))
            ml.append(s * (1.0 / NT))
            m2.append(_sum([(a - ml[-1]) * (a - ml[-1]) for a in xs]))
        yield
        mean = [jnp.broadcast_to(a, (8, 128)) * (1.0 / D) for a in tot]
        tot = [jnp.sum(b + ((a - m) * (a - m)) * float(NT), axis=1, keepdims=True)
               for a, b, m in zip(ml, m2, mean)]
        yield
        var = _round4([jnp.broadcast_to(a, (8, 128)) * (1.0 / D) for a in tot])
        var = _round4([a + EPS for a in var])
        sd = _round4([a * lax.rsqrt(a) for a in var])
        inv = [jnp.where(a == jnp.inf, 0.0, pltpu.reciprocal(b, full_range=False))
               for a, b in zip(var, sd)]
        r = None
        for t in range(NT):
            y = [a - m for a, m in zip(load(t), mean)]
            y = [a * b for a, b in zip(y, inv)]
            for s in range(4):
                xn[t, pl.ds(32 * i + 8 * s, 8), :] = y[s].astype(BF)
            a = [a * wrf[:, _col(t)] for a in y]
            r = a if r is None else [b + e for b, e in zip(r, a)]
        vpu_done(lax.bitcast_convert_type(_sum(r), U32))
        r = [jnp.sum(a, axis=1, keepdims=True) for a in r]
        st["xn"] = 32 * (i + 1)
        yield
        for s in range(4):
            st["r"][i // 32] = jnp.where(lane == (4 * i + s) % 128, r[s], st["r"][i // 32])
        vpu_done(lax.bitcast_convert_type(st["r"][i // 32], U32))

    def gating(i):
        half = paced(jnp.full((8, 128), 0.5, F32))
        half = jnp.concatenate([half] * 4, axis=0)
        for t in range(NT):
            a = _silu(_bf(xnu[t, pl.ds(16 * i, 16), :]).astype(F32), half)
            gate[t, pl.ds(32 * i, 32), :] = a
        vpu_done(lax.bitcast_convert_type(a[24:], U32))

    def product(task, k0, k1):
        half, k = pl.ds(task[1] * M // 2, M // 2), _col(k0, k1 - k0)
        wrap = gated if k0 == 0 else (lambda u: u)
        src = xnu if task[0] == "qkv" else obu
        a = _bf(wrap(jnp.concatenate([src[t, half, :] for t in range(k0, k1)], axis=1)))
        if task[0] == "qkv":
            return _nt(a, _bf(wt[task[2], pl.ds(task[3] * 64, 64), k]))
        return _nn(a, _bf(wop[pl.ds(k0 * 64, (k1 - k0) * 64), _col(task[2])]))

    def store_qkv(y, c, m, t):
        dst, off = ((qs, 0), (ks, HALO), (vs, HALO))[m]
        dst[t, pl.ds(off + c * M, M), :] = y
        if off and c == 0:
            dst[t, pl.ds(0, HALO), :] = jnp.broadcast_to(y[0:1, :], (HALO, 128))

    def store_out(s, c, t):
        rows = pl.ds(c * M, M)
        y = x_rows(t, c * M, M) + s * gate[t, rows, :]
        outb[rows, _col(t)] = y.astype(BF)
        pltpu.make_async_copy(outb.at[rows, _col(t)], out_hbm.at[rows, _col(t)], osem).start(
            priority=1)

    def attend(j):
        dep = st["mxu"][-1]
        for a in st["out"].get(j - BACK, []):
            dep = dep ^ a
        scale = after(jnp.full((8, 128), DH ** -0.5 * LOG2E, F32), dep)
        both = []
        for r0 in (16 * j, 16 * j + 8):
            win = [pl.ds(HALO + r0 - DIL * w, 8) for w in range(W)]
            q = [qs[t, pl.ds(r0, 8), :] * scale for t in range(NT)]
            p = [_sum([q[t] * ks[t, r, :] for t in range(NT)]) for r in win]
            p = [a + pltpu.roll(a, 64, 1) for a in p]
            p = [a + pltpu.roll(a, 32, 1) for a in p]
            row = lax.broadcasted_iota(I32, (8, 128), 0) + r0
            p = [jnp.where(row >= DIL * w, a, NEG * LOG2E) if r0 < DIL * w else a
                 for w, a in enumerate(p)]
            mx = functools.reduce(jnp.maximum, p)
            e = [jnp.exp2(a - mx) for a in p]
            inv = pltpu.reciprocal(_sum(e), full_range=False)
            o = [_sum([a * vs[t, r, :] for a, r in zip(e, win)]) * inv for t in range(NT)]
            for t in range(NT):
                ob[t, pl.ds(r0, 8), :] = o[t].astype(BF)
            both.append([lax.bitcast_convert_type(a, U32) for a in o[NO:]])
        st["out"][j] = [a ^ b for a, b in zip(*both)]
        vpu_done(st["out"][j][-1])

    def route():
        r = jnp.concatenate(_round2(*st["r"]), axis=1)
        key = jnp.where(r != r, -jnp.inf, r)
        slot = lax.broadcasted_iota(I32, (8, 256), 1)
        tok = slot * 8 + lax.broadcasted_iota(I32, (8, 256), 0)
        tok = tok.astype(F32)
        both = lambda f, a: f(f(a, axis=0, keepdims=True), axis=1, keepdims=True)
        full = lambda a: lax.bitcast_convert_type(jnp.broadcast_to(a, (8, 128)), U32)
        picks = []
        for _ in range(2):
            top = both(jnp.max, key)
            yield
            cand = key == top
            if picks:
                cand = cand & (tok != picks[0][0])
            idx = both(jnp.min, jnp.where(cand, tok, float(S)))
            yield
            vpu_done(full(idx))
            picks.append((idx, both(jnp.sum, jnp.where(tok == idx, r, 0.0))))
            key = jnp.where(tok == idx, -jnp.inf, key)
        picks = [(i.astype(I32), a) for i, a in picks]
        sidx = [jnp.squeeze(i) for i, _ in picks]
        base = [pl.multiple_of((i >> 3) * 8, 8) for i in sidx]
        src = [pl.multiple_of((i >> 4) * 8, 8) for i in sidx]
        yield
        row = lax.broadcasted_iota(I32, (16, 128), 0)
        odd = (lax.broadcasted_iota(I32, (8, 128), 0) & 1) == 1
        xs = []
        for t in range(NT):
            sel = [jnp.sum(jnp.where(row == (i & 15),
                                     _bf(xnu[t, pl.ds(b, 8), :]).astype(F32), 0.0),
                           axis=0, keepdims=True) for (i, _), b in zip(picks, src)]
            xs.append(jnp.where(odd, sel[1], sel[0]))
        for a in xs + [a for _, a in picks]:
            vpu_done(full(a))
        st["route"] = (picks, base, xs)

    def ffn():
        picks, base, xs = st["route"]
        lhs = lambda us: jnp.concatenate([paced(u, -3) for u in us], axis=1)

        def rhs(i, n0, n1, ts):
            rows = pl.ds(n0 * 64, min(n1 * 64, F // 2) - n0 * 64)
            return jnp.concatenate([_bf(wfu[i * NT + t, rows, :]) for t in ts], axis=1)

        hid = []
        for n0 in range(0, NF, 2):
            rem = {(i, n): _nt(lhs(xs[4:]), rhs(i, n, n + 1, [4]))
                   for n in (n0, n0 + 1) for i in range(2)}
            yield
            for n in (n0, n0 + 1):
                gu = []
                for i in range(2):
                    gu.append(_nt(lhs(xs[:4]), rhs(i, n, n + 1, range(4))) + rem[i, n])
                    yield
                g, u = [_round(a) for a in gu]
                hid.append(_round(_round(_silu(g)) * u))
        y = y4 = None
        for n in range(NF):
            a = _nn(lhs(hid[n:n + 1]), rhs(2, n, n + 1, range(4)))
            y = a if y is None else y + a
            yield
        for n0 in range(0, NF, 4):
            a = _nn(lhs(hid[n0:n0 + 4]), rhs(2, n0, n0 + 4, [4]))
            y4 = a if y4 is None else y4 + a
            yield
        y = _round(jnp.concatenate([y, y4], axis=1))
        assert st["gated"] == S // 32
        row = lax.broadcasted_iota(I32, (8, 128), 0)
        for j, (idx, val) in enumerate(picks):
            upd = _round(y[j:j + 1] * _round(jax.nn.sigmoid(val)))
            for t in range(NT):
                g = _silu(_round(xs[t][j:j + 1] + upd[:, t * 128:(t + 1) * 128]))
                b = pl.ds(base[j], 8)
                gate[t, b, :] = jnp.where(row == (idx & 7), g, gate[t, b, :])

    for cp in (wrcopy, xcopy[0], kcopy[0], kcopy[1], xcopy[1], xcopy[2], vcopy):
        cp.start()
    xcopy[0].wait()
    wrcopy.wait()
    wrf[...] = jnp.broadcast_to(wrb[...].astype(F32).reshape(1, D), (8, D))
    st["never"] = (lax.bitcast_convert_type(wrf[:, _col(0)], I32) & 0xFFFF) != 0
    started = XCUT[1] // 32
    live = [norm(i) for i in range(started)]
    while live:
        live = [g for g in live if not _advance(g)]
    for cp, a, b in zip(kcopy, KCUT[:-1], KCUT[1:]):
        cp.wait()
        for f in (prep_a, prep_b):
            for t in range(a // 128, b // 128):
                f(1, t)
    xcopy[1].wait()
    live = [norm(started + i) for i in range(M // 32)]
    started += M // 32
    live = [g for g in live if not _advance(g)]

    order = _slot_order()
    app = M // 16
    need = {t[1]: s - s % 4 for s, t in enumerate(order) if t[0] == "proj" and t[2] == 0}
    avail = {t[1]: s for s, t in enumerate(order) if t[0] == "qkv" and t[2:] == (0, NT - 1)}
    waits = {B1: [xcopy[2]], B2: [vcopy], B3: [xcopy[3], qcopy], FFN_AT: [fcopy]}
    starts = {B1: [xcopy[3], qcopy], F0: [fcopy]}
    arrived = {B1: (XCUT[3], LN1_DUE), B3: (XCUT[4], LN2_DUE)}
    extra = {}
    for t in range(NT):
        for s, f, args in ((B2 + t, prep_a, (2, t)), (B2 + 1 + t, prep_b, (2, t)),
                           (B3 + t, prep_a, (0, t)), (B3 + 2 + t, prep_b, (0, t)),
                           (FFN_AT + 5 * t, prep_wo, (t,))):
            extra.setdefault(s, []).append(functools.partial(f, *args))

    routeg, ffng = route(), ffn()
    route_done = ffn_done = False
    xrows, xdue = XCUT[2], LN0_DUE
    attended = 0
    lcredit = gcredit = acredit = 0.0
    for slot, task in enumerate(order):
        if slot % 4 == 0:
            for u in order[slot:slot + 4]:
                assert (st["xn"] >= (u[1] + 1) * M if u[0] == "qkv"
                        else attended >= (u[1] + 1) * app), (slot, u)
            rem = [product(u, 4, NT) for u in order[slot:slot + 4]]
        y = product(task, 0, 4) + rem[slot % 4]
        mxu_done(y[-8:])
        if task[0] == "qkv":
            store_qkv(y, *task[1:])
        else:
            assert ffn_done
            store_out(y, *task[1:])
        for cp in waits.get(slot, []):
            cp.wait()
        for cp in starts.get(slot, []):
            cp.start()
        xrows, xdue = arrived.get(slot, (xrows, xdue))

        if slot >= FFN_AT and not ffn_done:
            assert route_done
            ffn_done = _advance(ffng)
        if started == S // 32 and not live and not route_done and slot % RS == 0:
            route_done = _advance(routeg)
        lcredit = min(lcredit + (xrows // 32 - started) / max(xdue - slot, 1), 1.0)
        if lcredit >= 0.999 and started < xrows // 32:
            lcredit -= 1
            live.append(norm(started))
            started += 1
        live = [g for g in live if not _advance(g)]

        for lim, s0, s1 in ((XCUT[3] // 32, NT * NK, B3),
                            (S // 32, G0, G1)):
            if s0 <= slot and st["gated"] < lim:
                gcredit += (lim - st["gated"]) / max(s1 - slot, 1)
                gcredit = min(gcredit, 1.5)
                while gcredit >= 0.999 and st["gated"] < min(lim, st["xn"] // 32):
                    gcredit -= 1
                    gating(st["gated"])
                    st["gated"] += 1
                break

        ready = sum(app for c in avail if avail[c] + LAG <= slot)
        rate = max((c + 1) * app - attended for c in need) and max(
            ((c + 1) * app - attended) / max(need[c] - 3 - LAG - slot, 1) for c in need)
        acredit += rate if slot > LN2_DUE else min(rate, A1)
        while acredit >= PAIR and attended < ready:
            acredit -= PAIR
            for _ in range(PAIR):
                attend(attended)
                attended += 1
        acredit = min(acredit, PAIR)
        for f in extra.get(slot, []):
            f()
    pltpu.make_async_copy(outb, out_hbm, osem).wait()


@jax.jit
def pallas_recurrent_scan__sliding_local_dilated__moe_arch_mod__prompt_kernel(
    A_x, A_wqkv, A_wo, B_x, B_w_r, B_w_gate, B_w_up, B_w_down,
):
    del B_x
    hbm = pl.BlockSpec(memory_space=pltpu.HBM)
    V = pltpu.VMEM
    out = pl.pallas_call(
        _kernel,
        in_specs=[hbm] * 7,
        out_specs=hbm,
        out_shape=jax.ShapeDtypeStruct((S, D), BF),
        scratch_shapes=[
            [V((NT, b - a, 128), BF) for a, b in zip(XCUT[:-1], XCUT[1:])],
            [V((b - a, D), BF) for a, b in zip(KCUT[:-1], KCUT[1:])],
            V((D, D), BF), V((D, D), BF), V((D, D), BF),
            V((D,), BF),
            V((8, D), F32),
            V((3 * NT, F, 128), BF),
            V((4 * NT, D // 2 + 24, 128), U32),
            V((3, D // 2, D), U32),
            V((D // 2, D), U32),
            V((NT, S, 128), BF),
            V((NT, S, 128), F32),
            V((NT, S, 128), F32),
            V((NT, HALO + S, 128), F32),
            V((NT, HALO + S, 128), F32),
            V((NT, S, 128), BF),
            V((S, D), BF),
            pltpu.SemaphoreType.DMA((5 + len(XCUT),)),
            pltpu.SemaphoreType.DMA(()),
        ],
        compiler_params=pltpu.CompilerParams(vmem_limit_bytes=100 << 20),
        name="fused",
    )(A_x.reshape(S, D), A_wqkv, A_wo, B_w_r, B_w_gate.T, B_w_up.T, B_w_down)
    return out.reshape(1, S, D)
```

```python
import functools

import jax
import jax.numpy as jnp
import numpy as np
from jax import lax
from jax.experimental import pallas as pl
from jax.experimental.pallas import tpu as pltpu


S, D, F = 2048, 640, 1728
H, DH, W, DIL = 32, 20, 8, 2
NT = D // 128
NF = -(-F // 128)
HALO = 16
BF, F32, U32, I32 = jnp.bfloat16, jnp.float32, jnp.uint32, jnp.int32
LOG2E = 1.4426950408889634
NEG = -998244352.0
EPS = 1.0013580322265625e-05

M = 128
NC = S // M
NK = 6
XCUT = (0, 128, 384, NK * M, S)
KCUT = (0, 384, D)
B1 = 6
B2 = 20
B3 = 50
F0 = 40
FFN_AT = 180
LN_DUE = (4, 18, 156)
GATE_SPAN = (120, 234)
LAG = 2
REV = 9
BACK = 4
RATE = 0.43


def _round2(a, b):
    c = _round(jnp.concatenate([a, b], axis=1))
    return [c[:, :a.shape[1]], c[:, a.shape[1]:]]


def _round4(v):
    return _round2(v[0], v[1]) + _round2(v[2], v[3])


def _round(x):
    return x.astype(BF).astype(F32)


def _nt(a, b):
    return lax.dot_general(a, b, (((1,), (1,)), ((), ())), preferred_element_type=F32)


def _nn(a, b):
    return lax.dot_general(a, b, (((1,), (0,)), ((), ())), preferred_element_type=F32)


def _bf(u):
    return pltpu.bitcast(u, BF)


def _silu(x, half=0.5):
    h = x * half
    return h * jnp.tanh(h) + h


def _sum(xs):
    return functools.reduce(jnp.add, xs)


def _col(t, n=1):
    return pl.ds(t * 128, n * 128)


def _advance(g):
    return next(g, "end") == "end"


class _Copies:
    def __init__(self, pairs, sem):
        self.cs = [pltpu.make_async_copy(a, b, sem) for a, b in pairs]

    def start(self):
        for c in self.cs:
            c.start(priority=1)

    def wait(self):
        for c in self.cs:
            c.wait()


def _slot_order():
    tiles = lambda c, m: [("qkv", c, m, t) for t in range(NT)]
    order = [a for m in (1, 2, 0) for c in range(NK) for a in tiles(c, m)]
    order += [a for c in range(NK, NC) for m in (1, 2, 0) for a in tiles(c, m)]
    return order + [("proj", c, t) for c in range(NC) for t in range(NT)]


def _kernel(x_hbm, wqkv_hbm, wo_hbm, wr_hbm, wg_hbm, wu_hbm, wd_hbm, out_hbm,
            xb, kraw, vraw, qraw, oraw, wrb, wrf, wf, stage, wt, wop, xn, gate, qs, ks, vs, ob, outb,
            wsem, osem):
    xu = [b.bitcast(U32) for b in xb]
    xnu, obu, wfu = xn.bitcast(U32), ob.bitcast(U32), wf.bitcast(U32)
    xcopy = [_Copies([(x_hbm.at[pl.ds(a, b - a), _col(t)], xb[i].at[t]) for t in range(NT)],
                     wsem.at[6 + i])
             for i, (a, b) in enumerate(zip(XCUT[:-1], XCUT[1:]))]

    def x_rows(t, r0, n):
        i = max(j for j, a in enumerate(XCUT) if a <= r0)
        return _bf(xu[i][t, pl.ds((r0 - XCUT[i]) // 2, n // 2), :]).astype(F32)

    kcopy = [_Copies([(wqkv_hbm.at[pl.ds(a, b - a), _col(NT, NT)], kraw[i])], wsem.at[i])
             for i, (a, b) in enumerate(zip(KCUT[:-1], KCUT[1:]))]
    vcopy = _Copies([(wqkv_hbm.at[:, _col(2 * NT, NT)], vraw)], wsem.at[2])
    qcopy = _Copies([(wqkv_hbm.at[:, _col(0, NT)], qraw)], wsem.at[3])
    wrcopy = _Copies([(wr_hbm, wrb)], wsem.at[4])
    fcopy = _Copies([(wo_hbm, oraw)] + [
        (w.at[:, _col(t)], wf.at[i * NT + t])
        for i, w in enumerate((wg_hbm, wu_hbm, wd_hbm)) for t in range(NT)], wsem.at[5])

    lane = lax.broadcasted_iota(I32, (8, 128), 1)
    st = {"r": [jnp.zeros((8, 128), F32)] * 2, "xn": 0, "gated": 0,
          "mxu": [], "vpu": None, "hist": [], "out": {}}

    def after(v, dep):
        n = v.shape[1]
        return jnp.where(st["never"][:, :n], lax.bitcast_convert_type(dep, v.dtype)[:, :n], v)

    def mxu_done(v):
        v = lax.bitcast_convert_type(v, U32)
        st["mxu"].append(v ^ st["mxu"][-1] if st["mxu"] else v)

    def vpu_done(v):
        st["vpu"] = v if st["vpu"] is None else v ^ st["vpu"]

    def paced(v, age=-1):
        return after(v, st["mxu"][age]) if st["mxu"] else v

    def gated(u):
        st["hist"].append(st["vpu"])
        if len(st["hist"]) <= REV:
            return u
        head = jnp.concatenate([after(u[:8, :128], st["hist"][-1 - REV]), u[:8, 128:]], axis=1)
        return jnp.concatenate([head, u[8:]], axis=0)

    def permute_rows(src, dst, t):
        for d2 in range(DH // 2):
            u = src[pl.ds(d2, H // 2, stride=DH), :]
            v = src[pl.ds(d2 + DH // 2, H // 2, stride=DH), :]
            dst[pl.ds(H * d2, H // 2), _col(t)] = (u & np.uint32(0xFFFF)) | (v << 16)
            dst[pl.ds(H * d2 + H // 2, H // 2), _col(t)] = (u >> 16) | (v & np.uint32(0xFFFF0000))

    def prep_a(m, t):
        src, r0 = (qraw, 0) if m == 0 else (vraw, 0)
        if m == 1:
            i = int(t * 128 >= KCUT[1])
            src, r0 = kraw[i], KCUT[i]
        stage[m * NT + t, pl.ds(0, D // 2), :] = pltpu.bitcast(
            src[pl.ds(t * 128 - r0, 128), :].T, U32)

    def prep_b(m, t):
        permute_rows(stage.at[m * NT + t], wt.at[m], t)

    def prep_wo(t):
        stage[3 * NT + t, pl.ds(0, D // 2), :] = pltpu.bitcast(oraw[:, _col(t)], U32)
        permute_rows(stage.at[3 * NT + t], wop, t)

    def norm(i):
        x = [x_rows(t, 32 * i, 32) for t in range(NT)]
        x = [[a[8 * s:8 * s + 8] for s in range(4)] for a in x]
        x[0] = [paced(a) for a in x[0]]
        tot = [jnp.sum(_sum(xs), axis=1, keepdims=True) for xs in zip(*x)]
        yield
        mean = [jnp.broadcast_to(a, (8, 128)) * (1.0 / D) for a in tot]
        x = [[a - m for a, m in zip(xt, mean)] for xt in x]
        tot = [jnp.sum(_sum([a * a for a in xs]), axis=1, keepdims=True) for xs in zip(*x)]
        yield
        var = _round4([jnp.broadcast_to(a, (8, 128)) * (1.0 / D) for a in tot])
        var = _round4([a + EPS for a in var])
        sd = _round4([a * lax.rsqrt(a) for a in var])
        inv = [jnp.where(a == jnp.inf, 0.0, pltpu.reciprocal(b, full_range=False))
               for a, b in zip(var, sd)]
        r = None
        for t in range(NT):
            y = [a * b for a, b in zip(x[t], inv)]
            for s in range(4):
                xn[t, pl.ds(32 * i + 8 * s, 8), :] = y[s].astype(BF)
            a = [a * wrf[:, _col(t)] for a in y]
            r = a if r is None else [b + e for b, e in zip(r, a)]
        vpu_done(lax.bitcast_convert_type(_sum(r), U32))
        r = [jnp.sum(a, axis=1, keepdims=True) for a in r]
        st["xn"] = 32 * (i + 1)
        yield
        for s in range(4):
            st["r"][i // 32] = jnp.where(lane == (4 * i + s) % 128, r[s], st["r"][i // 32])
        vpu_done(lax.bitcast_convert_type(st["r"][i // 32], U32))

    def gating(i):
        half = paced(jnp.full((8, 128), 0.5, F32))
        half = jnp.concatenate([half] * 4, axis=0)
        for t in range(NT):
            a = _silu(_bf(xnu[t, pl.ds(16 * i, 16), :]).astype(F32), half)
            gate[t, pl.ds(32 * i, 32), :] = a
        vpu_done(lax.bitcast_convert_type(a[24:], U32))

    def product(task, k0, k1):
        half, k = pl.ds(task[1] * M // 2, M // 2), _col(k0, k1 - k0)
        wrap = gated if k0 == 0 else (lambda u: u)
        src = xnu if task[0] == "qkv" else obu
        a = _bf(wrap(jnp.concatenate([src[t, half, :] for t in range(k0, k1)], axis=1)))
        if task[0] == "qkv":
            return _nt(a, _bf(wt[task[2], pl.ds(task[3] * 64, 64), k]))
        return _nn(a, _bf(wop[pl.ds(k0 * 64, (k1 - k0) * 64), _col(task[2])]))

    def store_qkv(y, c, m, t):
        dst, off = ((qs, 0), (ks, HALO), (vs, HALO))[m]
        dst[t, pl.ds(off + c * M, M), :] = y
        if off and c == 0:
            dst[t, pl.ds(0, HALO), :] = jnp.broadcast_to(y[0:1, :], (HALO, 128))

    def store_out(s, c, t):
        rows = pl.ds(c * M, M)
        y = x_rows(t, c * M, M) + s * gate[t, rows, :]
        outb[rows, _col(t)] = y.astype(BF)
        pltpu.make_async_copy(outb.at[rows, _col(t)], out_hbm.at[rows, _col(t)], osem).start(
            priority=1)

    def attend(j):
        dep = st["mxu"][-1]
        for a in st["out"].get(j - BACK, []):
            dep = dep ^ a
        scale = after(jnp.full((8, 128), DH ** -0.5 * LOG2E, F32), dep)
        both = []
        for r0 in (16 * j, 16 * j + 8):
            win = [pl.ds(HALO + r0 - DIL * w, 8) for w in range(W)]
            q = [qs[t, pl.ds(r0, 8), :] * scale for t in range(NT)]
            p = [_sum([q[t] * ks[t, r, :] for t in range(NT)]) for r in win]
            p = [a + pltpu.roll(a, 64, 1) for a in p]
            p = [a + pltpu.roll(a, 32, 1) for a in p]
            row = lax.broadcasted_iota(I32, (8, 128), 0) + r0
            p = [jnp.where(row >= DIL * w, a, NEG * LOG2E) if r0 < DIL * w else a
                 for w, a in enumerate(p)]
            mx = functools.reduce(jnp.maximum, p)
            e = [jnp.exp2(a - mx) for a in p]
            inv = pltpu.reciprocal(_sum(e), full_range=False)
            o = [_sum([a * vs[t, r, :] for a, r in zip(e, win)]) * inv for t in range(NT)]
            for t in range(NT):
                ob[t, pl.ds(r0, 8), :] = o[t].astype(BF)
            both.append([lax.bitcast_convert_type(a, U32) for a in o[2:]])
        st["out"][j] = [a ^ b for a, b in zip(*both)]
        vpu_done(st["out"][j][-1])

    def route():
        r = jnp.concatenate(_round2(*st["r"]), axis=1)
        key = jnp.where(r != r, -jnp.inf, r)
        slot = lax.broadcasted_iota(I32, (8, 256), 1)
        tok = slot * 8 + lax.broadcasted_iota(I32, (8, 256), 0)
        tok = tok.astype(F32)
        both = lambda f, a: f(f(a, axis=0, keepdims=True), axis=1, keepdims=True)
        full = lambda a: lax.bitcast_convert_type(jnp.broadcast_to(a, (8, 128)), U32)
        picks = []
        for _ in range(2):
            top = both(jnp.max, key)
            yield
            cand = key == top
            if picks:
                cand = cand & (tok != picks[0][0])
            idx = both(jnp.min, jnp.where(cand, tok, float(S)))
            yield
            vpu_done(full(idx))
            picks.append((idx, both(jnp.sum, jnp.where(tok == idx, r, 0.0))))
            key = jnp.where(tok == idx, -jnp.inf, key)
        picks = [(i.astype(I32), a) for i, a in picks]
        sidx = [jnp.squeeze(i) for i, _ in picks]
        base = [pl.multiple_of((i >> 3) * 8, 8) for i in sidx]
        src = [pl.multiple_of((i >> 4) * 8, 8) for i in sidx]
        yield
        row = lax.broadcasted_iota(I32, (16, 128), 0)
        odd = (lax.broadcasted_iota(I32, (8, 128), 0) & 1) == 1
        xs = []
        for t in range(NT):
            sel = [jnp.sum(jnp.where(row == (i & 15),
                                     _bf(xnu[t, pl.ds(b, 8), :]).astype(F32), 0.0),
                           axis=0, keepdims=True) for (i, _), b in zip(picks, src)]
            xs.append(jnp.where(odd, sel[1], sel[0]))
        for a in xs + [a for _, a in picks]:
            vpu_done(full(a))
        st["route"] = (picks, base, xs)

    def ffn():
        picks, base, xs = st["route"]
        lhs = lambda us: jnp.concatenate([paced(u, -3) for u in us], axis=1)

        def rhs(i, n0, n1, ts):
            rows = pl.ds(n0 * 64, min(n1 * 64, F // 2) - n0 * 64)
            return jnp.concatenate([_bf(wfu[i * NT + t, rows, :]) for t in ts], axis=1)

        hid = []
        for n0 in range(0, NF, 2):
            rem = {(i, n): _nt(lhs(xs[4:]), rhs(i, n, n + 1, [4]))
                   for n in (n0, n0 + 1) for i in range(2)}
            yield
            for n in (n0, n0 + 1):
                gu = []
                for i in range(2):
                    gu.append(_nt(lhs(xs[:4]), rhs(i, n, n + 1, range(4))) + rem[i, n])
                    yield
                g, u = [_round(a) for a in gu]
                hid.append(_round(_round(_silu(g)) * u))
        y = y4 = None
        for n in range(NF):
            a = _nn(lhs(hid[n:n + 1]), rhs(2, n, n + 1, range(4)))
            y = a if y is None else y + a
            yield
        for n0 in range(0, NF, 4):
            a = _nn(lhs(hid[n0:n0 + 4]), rhs(2, n0, n0 + 4, [4]))
            y4 = a if y4 is None else y4 + a
            yield
        y = _round(jnp.concatenate([y, y4], axis=1))
        assert st["gated"] == S // 32
        row = lax.broadcasted_iota(I32, (8, 128), 0)
        for j, (idx, val) in enumerate(picks):
            upd = _round(y[j:j + 1] * _round(jax.nn.sigmoid(val)))
            for t in range(NT):
                g = _silu(_round(xs[t][j:j + 1] + upd[:, t * 128:(t + 1) * 128]))
                b = pl.ds(base[j], 8)
                gate[t, b, :] = jnp.where(row == (idx & 7), g, gate[t, b, :])

    for cp in (wrcopy, xcopy[0], kcopy[0], kcopy[1], xcopy[1], xcopy[2], vcopy):
        cp.start()
    xcopy[0].wait()
    wrcopy.wait()
    wrf[...] = jnp.broadcast_to(wrb[...].astype(F32).reshape(1, D), (8, D))
    st["never"] = (lax.bitcast_convert_type(wrf[:, _col(0)], I32) & 0xFFFF) != 0
    started = XCUT[1] // 32
    live = [norm(i) for i in range(started)]
    while live:
        live = [g for g in live if not _advance(g)]
    for cp, a, b in zip(kcopy, KCUT[:-1], KCUT[1:]):
        cp.wait()
        for f in (prep_a, prep_b):
            for t in range(a // 128, b // 128):
                f(1, t)
    xcopy[1].wait()
    live = [norm(started + i) for i in range(M // 32)]
    started += M // 32
    live = [g for g in live if not _advance(g)]

    order = _slot_order()
    app = M // 16
    need = {t[1]: s - s % 4 for s, t in enumerate(order) if t[0] == "proj" and t[2] == 0}
    avail = {t[1]: s for s, t in enumerate(order) if t[0] == "qkv" and t[2:] == (0, NT - 1)}
    waits = {B1: [xcopy[2]], B2: [vcopy], B3: [xcopy[3], qcopy], FFN_AT: [fcopy]}
    starts = {B1: [xcopy[3], qcopy], F0: [fcopy]}
    arrived = {B1: (XCUT[3], LN_DUE[1]), B3: (XCUT[4], LN_DUE[2])}
    extra = {}
    for t in range(NT):
        for s, f, args in ((B2 + t, prep_a, (2, t)), (B2 + 1 + t, prep_b, (2, t)),
                           (B3 + t, prep_a, (0, t)), (B3 + 2 + t, prep_b, (0, t)),
                           (FFN_AT + 5 * t, prep_wo, (t,))):
            extra.setdefault(s, []).append(functools.partial(f, *args))

    routeg, ffng = route(), ffn()
    route_done = ffn_done = False
    xrows, xdue = XCUT[2], LN_DUE[0]
    attended = 0
    lcredit = gcredit = acredit = 0.0
    for slot, task in enumerate(order):
        if slot % 4 == 0:
            for u in order[slot:slot + 4]:
                assert (st["xn"] >= (u[1] + 1) * M if u[0] == "qkv"
                        else attended >= (u[1] + 1) * app), (slot, u)
            rem = [product(u, 4, NT) for u in order[slot:slot + 4]]
        y = product(task, 0, 4) + rem[slot % 4]
        mxu_done(y[-8:])
        if task[0] == "qkv":
            store_qkv(y, *task[1:])
        else:
            assert ffn_done
            store_out(y, *task[1:])
        for cp in waits.get(slot, []):
            cp.wait()
        for cp in starts.get(slot, []):
            cp.start()
        xrows, xdue = arrived.get(slot, (xrows, xdue))

        if slot >= FFN_AT and not ffn_done:
            assert route_done
            ffn_done = _advance(ffng)
        if started == S // 32 and not live and not route_done and slot % 3 == 0:
            route_done = _advance(routeg)
        lcredit = min(lcredit + (xrows // 32 - started) / max(xdue - slot, 1), 1.0)
        if lcredit >= 0.999 and started < xrows // 32:
            lcredit -= 1
            live.append(norm(started))
            started += 1
        live = [g for g in live if not _advance(g)]

        for lim, s0, s1 in ((XCUT[3] // 32, NT * NK, B3),
                            (S // 32, *GATE_SPAN)):
            if s0 <= slot and st["gated"] < lim:
                gcredit += (lim - st["gated"]) / max(s1 - slot, 1)
                gcredit = min(gcredit, 1.5)
                while gcredit >= 0.999 and st["gated"] < min(lim, st["xn"] // 32):
                    gcredit -= 1
                    gating(st["gated"])
                    st["gated"] += 1
                break

        ready = sum(app for c in avail if avail[c] + LAG <= slot)
        rate = max([((c + 1) * app - attended) / max(need[c] - 3 - LAG - slot, 1)
                    for c in need] + [0.0])
        acredit += rate if slot > LN_DUE[2] else min(rate, RATE)
        while acredit >= 1 and attended < ready:
            acredit -= 1
            attend(attended)
            attended += 1
        acredit = min(acredit, 1)
        for f in extra.get(slot, []):
            f()
    pltpu.make_async_copy(outb, out_hbm, osem).wait()


@jax.jit
def pallas_recurrent_scan__sliding_local_dilated__moe_arch_mod__prompt_kernel(
    A_x, A_wqkv, A_wo, B_x, B_w_r, B_w_gate, B_w_up, B_w_down,
):
    del B_x
    hbm = pl.BlockSpec(memory_space=pltpu.HBM)
    V = pltpu.VMEM
    out = pl.pallas_call(
        _kernel,
        in_specs=[hbm] * 7,
        out_specs=hbm,
        out_shape=jax.ShapeDtypeStruct((S, D), BF),
        scratch_shapes=[
            [V((NT, b - a, 128), BF) for a, b in zip(XCUT[:-1], XCUT[1:])],
            [V((b - a, D), BF) for a, b in zip(KCUT[:-1], KCUT[1:])],
            V((D, D), BF), V((D, D), BF), V((D, D), BF),
            V((D,), BF),
            V((8, D), F32),
            V((3 * NT, F, 128), BF),
            V((4 * NT, D // 2 + 24, 128), U32),
            V((3, D // 2, D), U32),
            V((D // 2, D), U32),
            V((NT, S, 128), BF),
            V((NT, S, 128), F32),
            V((NT, S, 128), F32),
            V((NT, HALO + S, 128), F32),
            V((NT, HALO + S, 128), F32),
            V((NT, S, 128), BF),
            V((S, D), BF),
            pltpu.SemaphoreType.DMA((5 + len(XCUT),)),
            pltpu.SemaphoreType.DMA(()),
        ],
        compiler_params=pltpu.CompilerParams(vmem_limit_bytes=100 << 20),
        name="fused",
    )(A_x.reshape(S, D), A_wqkv, A_wo, B_w_r, B_w_gate.T, B_w_up.T, B_w_down)
    return out.reshape(1, S, D)
```
